```python
import os as _os
_os.environ.setdefault('JAX_PLATFORMS', 'cpu')
import jax
import jax.numpy as jnp

def _softmax(x, axis=-1):
    return jax.nn.softmax(x, axis=axis)

def _gelu(x):
    return jax.nn.gelu(x, approximate=True)

def _silu(x):
    return jax.nn.silu(x)

def _sigmoid(x):
    return jax.nn.sigmoid(x)

def _layernorm(x, axis=-1, eps=1e-05):
    m = jnp.mean(x, axis=axis, keepdims=True)
    v = jnp.var(x, axis=axis, keepdims=True)
    return (x - m) / jnp.sqrt(v + eps)

def _scatter_add(tgt, idx, src, axis=0):
    return tgt.at[idx].add(src)

def _segment_sum(src, seg, n):
    return jax.ops.segment_sum(src, seg, n)

class _Rng:

    def __init__(self, key):
        self._k = key

    def _next(self):
        self._k, sub = jax.random.split(self._k)
        return sub

    def normal(self, shape):
        return jax.random.normal(self._next(), shape, dtype=jnp.bfloat16)

    def randint(self, lo, hi, shape):
        return jax.random.randint(self._next(), shape, lo, hi, dtype=jnp.int32)

    def uniform(self, shape, lo=0.0, hi=1.0):
        return jax.random.uniform(self._next(), shape, jnp.bfloat16, lo, hi)

    def permutation(self, n):
        return jax.random.permutation(self._next(), n)
kernel_name = 'adaLN_cond__grouped_kv_mqa__swiglu_ffn__prompt'

def setup_inputs():
    _rng = _Rng(jax.random.key(int.from_bytes(__import__("os").urandom(4), "little")))
    _w = lambda a: (lambda t: t.astype(jnp.bfloat16) if jnp.issubdtype(t.dtype, jnp.floating) else t)(jnp.asarray(a))

    def _A_setup():
        B, S, D, H = (1, 2048, 576, 32)
        Dh = D // H
        return {'x': _w((lambda *s: _rng.normal(s) * 0.05)(B, S, D)), 'wq': _w((lambda *s: _rng.normal(s) * 0.05)(D, H * Dh)), 'wk': _w((lambda *s: _rng.normal(s) * 0.05)(D, Dh)), 'wv': _w((lambda *s: _rng.normal(s) * 0.05)(D, Dh)), 'wo': _w((lambda *s: _rng.normal(s) * 0.05)(H * Dh, D))}
    _A_in = _A_setup()

    def _B_setup():
        B, S, D, F = (1, 2048, 576, 4608)
        return {'x': _w((lambda *s: _rng.normal(s) * 0.05)(B, S, D)), 'w_gate': _w((lambda *s: _rng.normal(s) * 0.05)(D, F)), 'w_up': _w((lambda *s: _rng.normal(s) * 0.05)(D, F)), 'w_down': _w((lambda *s: _rng.normal(s) * 0.05)(F, D))}
    _B_in = _B_setup()
    return {'A_x': _A_in['x'], 'A_wq': _A_in['wq'], 'A_wk': _A_in['wk'], 'A_wv': _A_in['wv'], 'A_wo': _A_in['wo'], 'B_x': _B_in['x'], 'B_w_gate': _B_in['w_gate'], 'B_w_up': _B_in['w_up'], 'B_w_down': _B_in['w_down'], 'c': _w((lambda *s: _rng.normal(s) * 0.05)(1, 576) * 8.0), 'w_mod': _w((lambda *s: _rng.normal(s) * 0.05)(576, 6 * 576) * 576 ** (-0.5) * 8.0)}

def reference(A_x, A_wq, A_wk, A_wv, A_wo, B_x, B_w_gate, B_w_up, B_w_down, c, w_mod):

    def _A_ref(x, wq, wk, wv, wo):
        B, S, D = x.shape
        H = 32
        Dh = D // H
        q = (lambda x, *d: x.transpose(*d))((x @ wq).reshape(B, S, H, Dh), 0, 2, 1, 3)
        k = x @ wk
        v = x @ wv
        scores = jnp.einsum('bhqd,bkd->bhqk', q, k) * Dh ** (-0.5)
        p = _softmax(scores, axis=-1)
        o = jnp.einsum('bhqk,bkd->bhqd', p, v)
        return (lambda x, *d: x.transpose(*d))(o, 0, 2, 1, 3).reshape(B, S, H * Dh) @ wo

    def _B_ref(x, w_gate, w_up, w_down):
        g = _silu(x @ w_gate)
        u = x @ w_up
        return g * u @ w_down
    x = A_x
    mod = (_silu(c) @ w_mod).reshape(c.shape[0], 6, 1, -1)
    sa, ca, ga, sb, cb, gb = (mod[:, 0].copy(), mod[:, 1].copy(), mod[:, 2].copy(), mod[:, 3].copy(), mod[:, 4].copy(), mod[:, 5].copy())
    h = _layernorm(x, axis=-1) * (1 + ca) + sa
    x = x + ga * _A_ref(h, A_wq, A_wk, A_wv, A_wo)
    h = _layernorm(x, axis=-1) * (1 + cb) + sb
    x = x + gb * _B_ref(h, B_w_gate, B_w_up, B_w_down)
    return x
```

```python
import functools
import math

import jax
import jax.numpy as jnp
import numpy as np
from jax import lax
import jax.experimental.pallas as pl
import jax.experimental.pallas.tpu as pltpu

BF16 = jnp.bfloat16
F32 = jnp.float32

H = 32
EPS = 1e-5

NT = (((1,), (1,)), ((), ()))


def _dot(a, b):
    return jnp.dot(a, b, preferred_element_type=F32)


def _ln_t(x):
    n = x.shape[0]
    m = jnp.sum(x, axis=0, keepdims=True) * (1.0 / n)
    d = x - m
    v = jnp.sum(d * d, axis=0, keepdims=True) * (1.0 / n)
    return d * lax.rsqrt(v + EPS)


def make_kernel(S, D, F, TQ=512, KC=128, FC=512, scopes=False):
    Dh = D // H
    NQ = S // TQ
    NG = H // 4
    qscale = float(Dh ** -0.5 * math.log2(math.e))
    import contextlib
    scope = (lambda n: jax.named_scope(n)) if scopes else (lambda n: contextlib.nullcontext())

    def kernel(x_hbm, wq_hbm, wk_hbm, wv_hbm, wo_hbm, wg_hbm, wu_hbm, wd_hbm, c_hbm, wm_hbm,
               out_hbm,
               x_v, wq_v, wk_v, wv_v, wo_v, wg_v, wu_v, wd_v, c_v, wm_v,
               mod_v, wqkv_v, wot_v, ws_v, q_v, k_v, v_v, s_v, m_v, o_v, x1_v, h_v, a_v, acc_v, ob_v,
               sems, osems):
        cp_c = pltpu.make_async_copy(c_hbm, c_v, sems.at[0])
        cp_wm0 = pltpu.make_async_copy(wm_hbm.at[:, pl.ds(0, 2 * D)], wm_v.at[:, pl.ds(0, 2 * D)], sems.at[1])
        cp_x = pltpu.make_async_copy(x_hbm, x_v, sems.at[2])
        cp_wq = pltpu.make_async_copy(wq_hbm, wq_v, sems.at[3])
        cp_wk = pltpu.make_async_copy(wk_hbm, wk_v, sems.at[4])
        cp_wv = pltpu.make_async_copy(wv_hbm, wv_v, sems.at[5])
        cp_wm1 = pltpu.make_async_copy(wm_hbm.at[:, pl.ds(2 * D, 4 * D)], wm_v.at[:, pl.ds(2 * D, 4 * D)], sems.at[6])
        cp_wo = pltpu.make_async_copy(wo_hbm, wo_v, sems.at[7])
        cp_wg = pltpu.make_async_copy(wg_hbm, wg_v, sems.at[8])
        cp_wu = pltpu.make_async_copy(wu_hbm, wu_v, sems.at[9])
        cp_wd = pltpu.make_async_copy(wd_hbm, wd_v, sems.at[10])
        for cp in (cp_c, cp_wq, cp_wk, cp_wv, cp_wm0, cp_x):
            cp.start()

        def mod_cols(lo, n):
            c = c_v[...].astype(F32)
            sc = jnp.broadcast_to(c * jax.nn.sigmoid(c), (16, D)).astype(BF16)
            m = _dot(sc, wm_v[:, lo:lo + n])
            mod_v[lo:lo + n, :] = jnp.broadcast_to(m[0:1, :], (128, n)).T

        def transpose_w(w_v):
            w = w_v[...].astype(F32)
            return w.T

        with scope("prologue"):
            cp_wq.wait()
            wqkv_v[0:D, :] = (transpose_w(wq_v)).astype(BF16)
            cp_wk.wait()
            cp_wv.wait()
            zpad = jnp.zeros((32 - Dh, D), F32)
            wqkv_v[D:D + 32, :] = jnp.concatenate([wk_v[...].astype(F32), zpad], axis=0).astype(BF16)
            wqkv_v[D + 32:D + 64, :] = jnp.concatenate([wv_v[...].astype(F32), zpad], axis=0).astype(BF16)
            cp_c.wait()
            cp_wm0.wait()
            mod_cols(0, 2 * D)
            cp_x.wait()
            for cp in (cp_wm1, cp_wo, cp_wg, cp_wu, cp_wd):
                cp.start()

        def tile_mod(i):
            m = mod_v[i * D:(i + 1) * D, :]
            return jnp.concatenate([m] * (TQ // 128), axis=1)

        with scope("qkv"):
            for t in range(NQ):
                sl = slice(t * TQ, (t + 1) * TQ)
                x = x_v[:, sl].astype(F32)
                h = (_ln_t(x) * (1.0 + tile_mod(1)) + tile_mod(0)).astype(BF16)
                qkv = _dot(wqkv_v[...], h)
                q_v[t] = qkv[0:D] * qscale
                kt = jnp.concatenate([qkv[D:D + 32], jnp.zeros((96, TQ), F32)], axis=0)
                k_v[sl, :] = kt.T[:, 0:32].astype(BF16)
                row = lax.broadcasted_iota(jnp.int32, (24, TQ), 0)
                vt = qkv[D + 32:D + 56].astype(BF16).astype(F32)
                v_v[:, sl] = jnp.where(row == Dh, 1.0, vt)

        def load_q(t, g):
            qg = q_v[t, pl.ds(pl.multiple_of(g * 72, 8), 72), :]
            z = jnp.zeros((32 - Dh, TQ), F32)
            return [jnp.concatenate([qg[j * Dh:(j + 1) * Dh], z], axis=0).astype(BF16) for j in range(4)]

        def stage(q, s_dst, s_src, m_src):
            mx = None
            acc = None
            for c in range(S // KC):
                ks = slice(c * KC, (c + 1) * KC)
                if q is not None:
                    s = _dot(k_v[ks, :], q)
                    s_dst[ks, :] = s
                    cm = jnp.max(s.reshape(KC // 8, 8, TQ), axis=0)
                    mx = cm if mx is None else jnp.maximum(mx, cm)
                if s_src is not None:
                    p = jnp.exp2(s_src[ks, :] - m_src).astype(BF16)
                    o = _dot(v_v[:, ks], p)
                    acc = o if acc is None else acc + o
            if mx is not None:
                mx = jnp.max(mx, axis=0, keepdims=True)
            if acc is not None:
                acc = acc[0:Dh] / acc[Dh:Dh + 1]
            return mx, acc

        with scope("attn_pre"):
            m0, _ = stage(load_q(0, 0)[0], s_v.at[0], None, None)
            m_v[...] = m0

        def attn_body(i, carry):
            t = i // NG
            g = i % NG
            i2 = jnp.minimum(i + 1, NQ * NG - 1)
            qs = load_q(t, g)
            qn = load_q(i2 // NG, i2 % NG)[0]
            m0 = m_v[...]
            m1, o0 = stage(qs[1], s_v.at[1], s_v.at[0], m0)
            m2, o1 = stage(qs[2], s_v.at[0], s_v.at[1], m1)
            m3, o2 = stage(qs[3], s_v.at[1], s_v.at[0], m2)
            m4, o3 = stage(qn, s_v.at[0], s_v.at[1], m3)
            m_v[...] = m4
            o_v[t, pl.ds(pl.multiple_of(g * 72, 8), 72), :] = jnp.concatenate([o0, o1, o2, o3], axis=0)
            return carry

        with scope("attn"):
            lax.fori_loop(0, NQ * NG, attn_body, 0)

        with scope("ffn_prep"):
            cp_wm1.wait()
            mod_cols(2 * D, 4 * D)
            cp_wo.wait()
            wot_v[...] = transpose_w(wo_v).astype(BF16)
            cp_wg.wait()
            cp_wu.wait()
            cp_wd.wait()
            g0 = wg_v[448:512, :]
            g1 = wg_v[512:576, :]
            u0 = wu_v[448:512, :]
            u1 = wu_v[512:576, :]
            ws_v[0:64, :] = u0
            ws_v[64:128, :] = g1
            wg_v[448:512, :] = (g0.astype(F32) - u0.astype(F32)).astype(BF16)
            wu_v[448:512, :] = (u1.astype(F32) - g1.astype(F32)).astype(BF16)

        def gate_up(j):
            fs = pl.ds(pl.multiple_of(j * FC, FC), FC)
            sh = _dot(h_v[:, 640:768], ws_v[:, fs])
            g = _dot(h_v[:, 0:512], wg_v[0:512, fs]) + sh
            hu = jnp.concatenate([h_v[:, 0:384], h_v[:, 512:640]], axis=1)
            u = _dot(hu, wu_v[0:512, fs]) + sh
            return (g * jax.nn.sigmoid(g) * u).astype(BF16)

        def down(j, a):
            fs = pl.ds(pl.multiple_of(j * FC, FC), FC)
            return lax.dot_general(wd_v[:, fs], a, NT, preferred_element_type=F32)

        NF = F // FC

        def out_copy(t):
            return pltpu.make_async_copy(ob_v.at[t], out_hbm.at[:, pl.ds(pl.multiple_of(t * TQ, TQ), TQ)], osems.at[t])

        def ffn_tile(t, carry):
            a = _dot(wot_v[...], o_v[t].astype(BF16))
            x1 = x_v[:, pl.ds(pl.multiple_of(t * TQ, TQ), TQ)].astype(F32) + tile_mod(2) * a
            x1_v[...] = x1
            h = _ln_t(x1) * (1.0 + tile_mod(4)) + tile_mod(3)
            hx = jnp.concatenate([h[0:512], h[384:448], h[512:576], h[448:576]], axis=0)
            h_v[...] = hx.T.astype(BF16)
            a_v[0] = gate_up(0)
            acc_v[...] = jnp.zeros_like(acc_v)

            def body(j, c):
                a_v[(j + 1) % 2] = gate_up(j + 1)
                acc_v[...] += down(j, a_v[j % 2])
                return c

            lax.fori_loop(0, NF - 1, body, 0)
            y = acc_v[...] + down(NF - 1, a_v[(NF - 1) % 2])
            ob_v[t] = (x1_v[...] + tile_mod(5) * y).astype(BF16)
            out_copy(t).start()
            return carry

        with scope("ffn"):
            lax.fori_loop(0, NQ, ffn_tile, 0)
            for t in range(NQ):
                out_copy(t).wait()

    scratch = [
        pltpu.VMEM((D, S), BF16), pltpu.VMEM((D, D), BF16), pltpu.VMEM((Dh, D), BF16), pltpu.VMEM((Dh, D), BF16),
        pltpu.VMEM((D, D), BF16), pltpu.VMEM((D, F), BF16), pltpu.VMEM((D, F), BF16), pltpu.VMEM((D, F), BF16),
        pltpu.VMEM((1, D), BF16), pltpu.VMEM((D, 6 * D), BF16),
        pltpu.VMEM((6 * D, 128), F32),
        pltpu.VMEM((D + 64, D), BF16),
        pltpu.VMEM((D, D), BF16),
        pltpu.VMEM((128, F), BF16),
        pltpu.VMEM((NQ, D, TQ), F32),
        pltpu.VMEM((S, 32), BF16),
        pltpu.VMEM((24, S), F32),
        pltpu.VMEM((2, S, TQ), F32),
        pltpu.VMEM((1, TQ), F32),
        pltpu.VMEM((NQ, D, TQ), F32),
        pltpu.VMEM((D, TQ), F32),
        pltpu.VMEM((TQ, 768), BF16),
        pltpu.VMEM((2, TQ, FC), BF16),
        pltpu.VMEM((D, TQ), F32),
        pltpu.VMEM((NQ, D, TQ), BF16),
        pltpu.SemaphoreType.DMA((11,)),
        pltpu.SemaphoreType.DMA((NQ,)),
    ]
    return kernel, scratch


def build(**cfg):
    flags = cfg.pop("flags", None)

    def fn(A_x, A_wq, A_wk, A_wv, A_wo, B_x, B_w_gate, B_w_up, B_w_down, c, w_mod):
        _, S, D = A_x.shape
        F = B_w_gate.shape[1]
        kernel, scratch = make_kernel(S, D, F, **cfg)
        out_t = pl.pallas_call(
            kernel,
            in_specs=[pl.BlockSpec(memory_space=pl.ANY)] * 10,
            out_specs=pl.BlockSpec(memory_space=pl.ANY),
            out_shape=jax.ShapeDtypeStruct((D, S), A_x.dtype),
            scratch_shapes=scratch,
            compiler_params=pltpu.CompilerParams(vmem_limit_bytes=110 * 2 ** 20, flags=flags),
            name="adaln_block",
        )(A_x[0].T, A_wq, A_wk.T, A_wv.T, A_wo, B_w_gate, B_w_up, B_w_down.T, c, w_mod)
        return out_t.T[None]

    return fn


pallas_adaLN_cond__grouped_kv_mqa__swiglu_ffn__prompt_kernel = jax.jit(build())
```

```python
import contextlib
import functools
import math

import jax
import jax.numpy as jnp
from jax import lax
import jax.experimental.pallas as pl
import jax.experimental.pallas.tpu as pltpu

BF16 = jnp.bfloat16
F32 = jnp.float32
U32 = jnp.uint32

H = 32
EPS = 1e-5
L = 128
SAFE_LOG2 = 60.0


def _dot(a, b):
    return jnp.dot(a, b, preferred_element_type=F32)


def _bc(x):
    return pltpu.bitcast(x, BF16)


def _pack2(lo, hi):
    return pltpu.pack_elementwise([lo, hi], packed_dtype=BF16)


def _unpack2(x):
    return [pltpu.unpack_elementwise(x, index=i, packed_dtype=BF16, unpacked_dtype=F32) for i in range(2)]


def _pack(s):
    n = s.shape[0] // 16
    s = s.reshape(n, 2, 8, s.shape[1])
    return _pack2(s[:, 0].reshape(n * 8, -1), s[:, 1].reshape(n * 8, -1))


def _even_odd(even, odd):
    n = even.shape[0] // 8
    return jnp.stack([even.reshape(n, 8, -1), odd.reshape(n, 8, -1)], axis=1).reshape(16 * n, -1)


def _to_packed(x):
    return pltpu.bitcast(x.astype(BF16), U32)


def _st_a(a):
    (a11, a12), (a21, a22) = a
    return [a11 + a22, a21 + a22, a11, a22, a11 + a12, a21 - a11, a12 - a22]


def _st_b(b):
    (b11, b12), (b21, b22) = b
    return [b11 + b22, b11, b12 - b22, b21 - b11, b22, b11 + b12, b21 + b22]


def _st_c(m):
    m1, m2, m3, m4, m5, m6, m7 = m
    return [[m1 + m4 - m5 + m7, m3 + m5], [m2 + m4, m1 - m2 + m3 + m6]]


def _two_level(st, x):
    l1 = [[st([[x[r][c], x[r][c + 2]], [x[r + 2][c], x[r + 2][c + 2]]]) for c in range(2)] for r in range(2)]
    return [st([[l1[0][0][i], l1[0][1][i]], [l1[1][0][i], l1[1][1][i]]]) for i in range(7)]


def _norm_steps(load, n, emit, rows):
    st = {}

    def fold(key, x):
        x = jnp.sum(x.reshape(-1, 8, x.shape[1]), axis=0)
        st[key] = st[key] + x if key in st else x

    def total(key):
        return jnp.sum(st[key], axis=0, keepdims=True) * (1.0 / n)

    def sums(r, pin):
        fold("sum", load(r, 64))
        if r + 64 == n:
            st["mean"] = jnp.broadcast_to(total("sum"), st["sum"].shape)

    def squares(r, pin):
        d = load(r, 64) - jnp.concatenate([pin(st["mean"])] * 8, axis=0)
        fold("sq", d * d)
        if r + 64 == n:
            st["rstd"] = lax.rsqrt(total("sq") + EPS)

    def write(r, pin):
        mean = jnp.concatenate([pin(st["mean"])] * 2, axis=0)
        emit(r, lambda r0: (load(r0, 16) - mean) * st["rstd"])

    return ([functools.partial(sums, r) for r in range(0, n, 64)]
            + [functools.partial(squares, r) for r in range(0, n, 64)]
            + [functools.partial(write, r) for r in rows])


def _run(steps):
    for step in steps:
        step(lambda x: x)


class _Filler:
    def __init__(self, never, cycles, *streams):
        self.never = never
        self.now = 0
        due = [(e * cycles // len(st), n, e, step) for n, st in enumerate(streams) for e, step in enumerate(st)]
        self.due = sorted(due, key=lambda d: d[:3], reverse=True)

    def tick(self, res, cycles):
        while self.due and self.due[-1][0] < self.now + cycles:
            at, _, _, step = self.due.pop()
            r = 8 * ((at - self.now) * (res.shape[0] // 8) // cycles)
            step(functools.partial(self.pin, res[r:r + 8, 0:L]))
        self.now += cycles

    def pin(self, mark, x):
        tile = lambda a: jnp.concatenate([jnp.concatenate([a] * (x.shape[1] // L), axis=1)] * (x.shape[0] // 8), axis=0)
        if x.dtype != mark.dtype:
            mark = pltpu.bitcast(mark, x.dtype)
        return jnp.where(tile(self.never), tile(mark), x)


def make_kernel(S, D, F, NV0=288, NV1=320, NVP=0, HG=56, HD=56, RB=64, UG=6, scopes=False, force_exact=False,
                NK=2, DS=5, htail=100, atail=0, WT=(40, 16), OR=144):
    TQ = 4 * L
    Dh = D // H
    NQ = S // TQ
    NG = H // 4
    NC = S // L
    NU = F // (4 * L)
    GI = NU * L // (RB * UG)
    assert HG % 4 == 0 and HD % 4 == 0 and (GI * HG + HD) % H == 0
    NH = 16 * NK * (GI * HG + HD) // H
    NB = (NQ + 1) * L
    KB = 16 * NK
    assert max(NV0, NV1 + NH) <= NB
    qscale = float(Dh ** -0.5 * math.log2(math.e))
    scope = (lambda n: jax.named_scope(n)) if scopes else (lambda n: contextlib.nullcontext())

    def kernel(x_hbm, wq_hbm, wk_hbm, wv_hbm, wo_hbm, wg_hbm, wu_hbm, wd_hbm, c_hbm, wm_hbm,
               out_hbm,
               x_v, wq_v, wo_v, raw_v, wm_v,
               mod_v, h_v, n_v, kx_v, wqkv_v, wot_v, q_v, k_v, kb_v, v_v, p_v, pp_v, o_v,
               wt_v, wa_v, ws_v, wdc_v, x1_v, hb_v, ab_v, ob_v, z_v, wk_v, wv_v, c_v,
               sems, xsems, wsems, osems):
        cp_c = pltpu.make_async_copy(c_hbm, c_v, sems.at[0])
        cp_wm0 = pltpu.make_async_copy(wm_hbm.at[:, pl.ds(0, 2 * D)], wm_v.at[:, pl.ds(0, 2 * D)], sems.at[1])
        cp_wq = pltpu.make_async_copy(wq_hbm, wq_v, sems.at[2])
        cp_wk = pltpu.make_async_copy(wk_hbm, wk_v, sems.at[3])
        cp_wv = pltpu.make_async_copy(wv_hbm, wv_v, sems.at[4])
        cp_wm1 = pltpu.make_async_copy(wm_hbm.at[:, pl.ds(2 * D, 4 * D)], wm_v.at[:, pl.ds(2 * D, 4 * D)], sems.at[5])
        cp_wo = pltpu.make_async_copy(wo_hbm, wo_v, sems.at[6])

        def x_copy(t):
            return pltpu.make_async_copy(x_hbm.at[:, pl.ds(pl.multiple_of(t * TQ, TQ), TQ)], x_v.at[t], xsems.at[t])

        def raw_copies(u):
            cols = pl.ds(pl.multiple_of(u * 4 * L, 4 * L), 4 * L)
            return [pltpu.make_async_copy(w.at[:, cols], raw_v.at[u % 3, i], wsems.at[u % 3, i])
                    for i, w in enumerate((wg_hbm, wu_hbm, wd_hbm))]

        def loop(n, f):
            def body(i, carry):
                with scope("it_%s_%d" % (f.__name__, n)):
                    f(i)
                return carry
            lax.fori_loop(0, n, body, 0)

        for cp in (cp_c, cp_wq, cp_wk, cp_wv, cp_wm0, x_copy(0)):
            cp.start()

        def mod_cols(first, affine):
            c = c_v[...].astype(F32)
            sc = jnp.broadcast_to(c * jax.nn.sigmoid(c), (16, D)).astype(BF16)
            m = _dot(sc, wm_v[:, first * D:(first + len(affine)) * D])
            m = jnp.broadcast_to(m[0:1, :], (L, m.shape[1])).T
            for i, (a, b) in enumerate(affine):
                mod_v[first + i] = m[i * D:(i + 1) * D] * a + b

        def mod(i, r, n, w):
            return jnp.concatenate([mod_v[i, r:r + n, :]] * w, axis=1)

        def modulate_steps(t, slot):
            def emit(r, norm):
                h_v[slot, r:r + 16, :] = (norm(r) * mod(1, r, 16, 4) + mod(0, r, 16, 4)).astype(BF16)
            return _norm_steps(lambda r, n: x_v[t, r:r + n, :].astype(F32), D, emit, range(0, D, 16))

        with scope("prologue"):
            z_v[...] = jnp.zeros_like(z_v)
            n_v[...] = jnp.zeros_like(n_v)
            for cp in (cp_wq, cp_wk, cp_wv):
                cp.wait()
            wqkv_v[0:D, :] = wq_v[...].T
            zpad = jnp.zeros((24 - Dh, D), F32)
            wqkv_v[D:D + 48, :] = jnp.concatenate(
                [wk_v[...].astype(F32), zpad, wv_v[...].astype(F32), zpad], axis=0).astype(BF16)
            cp_c.wait()
            cp_wm0.wait()
            x_copy(1).start()
            mod_cols(0, [(1.0, 0.0), (1.0, 1.0)])
            x_copy(0).wait()
            for cp in [x_copy(t) for t in range(2, NQ)] + [cp_wm1, cp_wo] + raw_copies(0):
                cp.start()
            _run(modulate_steps(0, 0))

        def spread_steps(kt, c):
            def spread(d, pin):
                rows = jnp.broadcast_to(kt[d:d + 1, :], (L - 8, L))
                blk = jnp.concatenate([pin(rows[0:8]), rows], axis=0).astype(BF16).T
                return _unpack2(pltpu.bitcast(blk, U32))

            def step(d, pin):
                (a11, a21), (a12, a22) = spread(d, pin), spread(d + Dh // 2, pin)
                s1 = a21 + a22
                s2 = s1 - a11
                for p, a in enumerate((a11, a12, a12 - s2, -a22, s1, s2, a11 - a21)):
                    for r in range(8):
                        kb_v[8 * c + r, 9 * p + d] = a[8 * r:8 * r + 8]
            return [functools.partial(step, d) for d in range(Dh // 2)]

        def project(t):
            @pl.when(t + 1 < NQ)
            def _():
                x_copy(jnp.minimum(t + 1, NQ - 1)).wait()

            h = h_v[t % 2]
            kv = _dot(wqkv_v[D:D + 48, :], h).astype(BF16).astype(F32)
            kt, vt = kv[0:24], kv[24:48]

            kx_v[0:24, :] = kt[:, TQ - 2 * L:TQ - L]
            fill = _Filler(z_v[...] != 0, D - 32, spread_steps(kt[:, TQ - L:], t + 1),
                           modulate_steps(jnp.minimum(t + 1, NQ - 1), (t + 1) % 2))
            R = D // 4
            q2 = n_v[0, 0:1, :]
            for r in range(4):
                q = _dot(wqkv_v[r * R:(r + 1) * R, :], h)
                fill.tick(q, R)
                q = (q * qscale).astype(BF16).astype(F32)
                up = pltpu.roll(q, R - Dh // 2, axis=0)
                t1 = q[:, 2 * L:] - q[:, :2 * L]
                t2 = up[:, 2 * L:] - t1
                qx = jnp.concatenate([q, t2 - up[:, :2 * L], t1, t2, up[:, 2 * L:] - q[:, 2 * L:]], axis=1)
                q_v[pl.ds(t * NG + 2 * r, 2)] = qx.reshape(2, 4 * Dh, 3 * TQ)
                qq = q * q
                for hh in range(R // Dh):
                    q2 = jnp.maximum(q2, jnp.sum(qq[hh * Dh:(hh + 1) * Dh], axis=0, keepdims=True))
            n_v[0, 0:1, :] = q2
            n_v[1, 0:1, :] = jnp.maximum(n_v[1, 0:1, :], jnp.sum(kt * kt, axis=0, keepdims=True))
            n_v[2, 0:1, :] = jnp.maximum(n_v[2, 0:1, :], jnp.max(jnp.abs(vt), axis=0, keepdims=True))
            kn = jnp.concatenate([kt, jnp.zeros((L - 24, TQ), F32)], axis=0).astype(BF16).T
            kn = _to_packed(_even_odd(*_unpack2(pltpu.bitcast(kn, U32))))[:, 0:32]
            row = lax.broadcasted_iota(jnp.int32, (24, TQ), 0)
            vn = jnp.where(row == Dh, 1.0, vt)
            for c in range(4):
                at = 3 * t + c if c < 3 else 3 * NQ + t
                k_v[pl.ds(pl.multiple_of(at * (L // 2), L // 2), L // 2), :] = kn[c * L // 2:(c + 1) * L // 2]
                v_v[at] = vn[:, c * L:(c + 1) * L]

        with scope("qkv"):
            loop(NQ, project)
            for cp in raw_copies(1):
                cp.start()
            cp_wm1.wait()
            cp_wo.wait()
            mod_cols(2, [(1.0, 0.0), (0.5, 0.0), (0.5, 0.5), (2.0, 0.0)])
            wot_v[...] = wo_v[...].T
            bound = jnp.max(n_v[0, 0:1, :], axis=1, keepdims=True) * n_v[1, 0:1, :]
            ok = jnp.logical_and(bound <= SAFE_LOG2 ** 2, n_v[2, 0:1, :] <= 2.0 ** 50)
            safe = jnp.max(jnp.where(ok, 0.0, 1.0)) < (-1.0 if force_exact else 0.5)

        def prep_wait(u):
            for cp in raw_copies(u):
                cp.wait()

            @pl.when(u + 2 < NU)
            def _():
                for cp in raw_copies(jnp.minimum(u + 2, NU - 1)):
                    cp.start()

        def prep_steps(u):
            slot = u % 3
            lane = lax.broadcasted_iota(jnp.int32, (8, L), 1)

            def transpose(w, half, kind, pin):
                k0 = half * (D // 2)
                rows = lambda r, m, n: raw_v[slot, w, k0 + r:k0 + r + m, n * L:(n + 1) * L]
                if kind < 4:
                    blk = rows(0, L, kind)
                elif kind < 8:
                    blk = jnp.concatenate([rows(L if m == kind - 4 else 160 + 32 * m, 32, kind - 4) for m in range(4)], axis=0)
                else:
                    blk = jnp.concatenate([rows(160 + 32 * m, 32, m) for m in range(4)], axis=0)
                blk = pltpu.bitcast(blk, U32)
                blk = jnp.concatenate([pin(blk[0:8]), blk[8:]], axis=0)
                wt_v[w, half, kind] = pltpu.bitcast(_bc(blk).T, U32)

            def combine(kind, r, pin):
                def operand(w, half):
                    x = _unpack2(pin(wt_v[w, half, kind, r:r + 8, :]))
                    if 4 <= kind < 8:
                        sh = _unpack2(jnp.where(lane // 32 == kind - 4, 0, wt_v[w, half, 8, r:r + 8, :]))
                        x = [x[0] - sh[0], x[1] - sh[1]]
                    return x
                x = [[operand(w, half) for half in range(2)] for w in range(2)]
                y = [_st_a([[x[w][half][e] for half in range(2)] for w in range(2)]) for e in range(2)]
                rows = pl.ds(pl.multiple_of(u * (L // 2) + r, 8), 8)
                for i in range(7):
                    if kind == 8:
                        ws_v[i, rows, :] = _pack2(y[0][i], y[1][i])
                    else:
                        wa_v[i, kind % 4, rows, kind // 4 * L:(kind // 4 + 1) * L] = _pack2(y[0][i], y[1][i])

            outer = {}

            def down_outer(r, a, b, pin):
                def operand(q, n):
                    r0 = q * (D // 4) + 2 * r
                    return _unpack2(pin(pltpu.bitcast(raw_v[slot, 2, r0:r0 + 16, n * L:(n + 1) * L], U32)))
                d = [[operand(a + 2 * q, 2 * b + n) for n in range(2)] for q in range(2)]
                outer[a, b] = [_st_a([[d[q][n][e] for n in range(2)] for q in range(2)]) for e in range(2)]

            def down_inner(r, i, pin):
                y = [_st_a([[(pin if a == b else lambda x: x)(outer[a, b][e][i]) for b in range(2)] for a in range(2)])
                     for e in range(2)]
                for k in range(7):
                    wdc_v[7 * i + k, u, r:r + 8, :] = _pack2(y[0][k], y[1][k])

            down_steps = []
            for r in range(0, D // 8, 8):
                down_steps += [functools.partial(down_outer, r, a, b) for a in range(2) for b in range(2)]
                down_steps += [functools.partial(down_inner, r, i) for i in range(7)]

            gate_up_steps = []
            kinds = [8, 0, 1, 2, 3, 4, 5, 6, 7]
            for n in range(10):
                if n < 9:
                    gate_up_steps += [functools.partial(transpose, w, half, kinds[n]) for w in range(2) for half in range(2)]
                if n > 0:
                    gate_up_steps += [functools.partial(combine, kinds[n - 1], r) for r in range(0, L // 2, 8)]
            return (gate_up_steps + down_steps,)

        def vpu_steps(i, j, b, store):
            n = Dh // 2
            st = {}
            q_at = [(0, 0), (n, 0), (n, 2), (0, 4), (0, 6), (0, 8), (0, 10)]

            def step(name, p, start, d0, pin):
                for d in range(d0, min(d0 + DS, n)):
                    r, l = j * Dh + q_at[p][0] + d, q_at[p][1]
                    k = jnp.concatenate([kb_v[b + m, n * p + d] for m in range(NK)], axis=0)
                    q = jnp.concatenate([jnp.broadcast_to(q_v[i, r:r + 1, m * L:(m + 1) * L], (8, L))
                                         for m in (l, l + 1)], axis=1)
                    t = jnp.concatenate([k, k], axis=1) * jnp.concatenate([pin(q) if d == d0 else q] * NK, axis=0)
                    prev = name if d else start
                    st[name] = t if prev is None else st[prev] + t
                if d0 + DS < n:
                    return
                if name == "u6":
                    store(slice(0, 2 * L), _pack2(jnp.exp2(st["u1"]), jnp.exp2(st["u6"])))
                elif name == "p5":
                    st["u7"], st["u4"] = st["u3"] + st["p5"], st["u2"] + st["p5"]
                elif name == "u5":
                    store(slice(2 * L, 4 * L), _pack2(jnp.exp2(st["u5"]), jnp.exp2(st["u7"])))
            plan = [("p1", 0, None), ("u1", 1, "p1"), ("u2", 5, "p1"), ("u3", 6, "u2"), ("u6", 3, "u3"),
                    ("p5", 4, None), ("u5", 2, "u4")]
            return [functools.partial(step, *p, d0) for p in plan for d0 in range(0, n, DS)]

        def stage(i, j, dst, src, nv, nh, hprev, *extra):
            z = jnp.zeros((32 - Dh, TQ), F32)
            q = jnp.concatenate([q_v[i, j * Dh:(j + 1) * Dh, 0:TQ], z], axis=0).astype(BF16)
            nm = S - nv - nh
            steps = []
            for k0 in range(nm, nm + nv, KB):
                def store(cols, p, k0=k0):
                    dst[k0 // 2:(k0 + KB) // 2, cols] = p
                steps += vpu_steps(i, j, (k0 - (S - NB)) // 16, store)
            fill = _Filler(z_v[...] != 0, nm + (24 * NC if src is not None else 0) - (atail if j == 0 else 0), steps, *extra)
            acc = None
            for c in range(NC):
                lo, hi = 16 * (c * (nm // 16) // NC), 16 * ((c + 1) * (nm // 16) // NC)
                s = _dot(_bc(k_v[lo // 2:hi // 2, :]), q)
                dst[lo // 2:hi // 2, :] = _pack(jnp.exp2(s))
                fill.tick(s, hi - lo)
                if src is not None:
                    k0, k1, kh = c * L, (c + 1) * L, S - nh
                    parts = []
                    if k0 < kh:
                        parts.append(src[k0 // 2:min(k1, kh) // 2, :])
                    if k1 > kh:
                        parts.append(pp_v[hprev, (max(k0, kh) - kh) // 2:(k1 - kh) // 2, :])
                    o = _dot(v_v[c], _bc(jnp.concatenate(parts, axis=0)))
                    acc = o if acc is None else acc + o
                    fill.tick(o, 24)
            return acc

        def attn_group(i, g, nv, nh, *extra):
            i2 = jnp.minimum(i + 1, NQ * NG - 1)
            for j in range(4):
                nxt = (i, j + 1) if j < 3 else (i2, 0)
                share = [st[j * len(st) // 4:(j + 1) * len(st) // 4] for st in extra]
                o_v[4 * g + j] = stage(*nxt, p_v.at[(j + 1) % 2], p_v.at[j % 2], nv, nh, 4 * g + j, *share)

        def exact_block(t, n):
            hh, cols = n // 4, pl.ds(pl.multiple_of(n % 4 * L, L), L)
            q = q_v[t * NG + hh // 4, 0:Dh, cols]
            for j in range(1, 4):
                q = jnp.where(hh % 4 == j, q_v[t * NG + hh // 4, j * Dh:(j + 1) * Dh, cols], q)
            s = _dot(_bc(k_v[...]), jnp.concatenate([q, jnp.zeros((32 - Dh, L), F32)], axis=0).astype(BF16))
            p = _pack(jnp.exp2(s - jnp.max(s, axis=0, keepdims=True)))
            o_v[hh, :, cols] = _dot(jnp.concatenate([v_v[c] for c in range(NC)], axis=1), _bc(p))

        with scope("attn0"):
            @pl.when(safe)
            def _():
                prep_wait(0)
                stage(0, 0, p_v.at[0], None, NVP, 0, 0, *prep_steps(0), spread_steps(kx_v[0:24, :], 0))

                def body(g):
                    prep_wait(g + 1)
                    attn_group(g, g, NV0, 0, *prep_steps(g + 1))
                loop(NG, body)

            @pl.when(jnp.logical_not(safe))
            def _():
                def body(u):
                    prep_wait(u)
                    for steps in prep_steps(u):
                        _run(steps)
                loop(NU, body)

        def Host(t, first, count, cycles):
            steps = []
            for e in range(count):
                b, hh = (first + e) // H, (first + e) % H

                def store(cols, p, b=b, hh=hh):
                    pp_v[hh, pl.ds(pl.multiple_of(b * (KB // 2), 8), KB // 2), cols] = p
                steps += vpu_steps(jnp.minimum(t + 1, NQ - 1) * NG + hh // 4, e % 4, (NB - NH) // 16 + b * NK, store)
            return _Filler(z_v[...] != 0, cycles - htail, steps)

        def out_copy(t):
            return pltpu.make_async_copy(ob_v.at[t], out_hbm.at[:, pl.ds(pl.multiple_of(t * TQ, TQ), TQ)], osems.at[t])

        def tile(t):
            with scope("attn"):
                @pl.when(safe)
                def _():
                    @pl.when(t > 0)
                    def _():
                        loop(NG, lambda g: attn_group(t * NG + g, g, NV1, NH))

                @pl.when(jnp.logical_not(safe))
                def _():
                    loop(4 * H, lambda n: exact_block(t, n))

            with scope("oproj"):
                inv = [1.0 / o_v[g:g + 8, Dh, :] for g in range(0, H, 8)]
                steps = []
                for pair in range(2):
                    cols = slice(2 * pair * L, 2 * (pair + 1) * L)
                    o = jnp.concatenate([o_v[hh, 0:Dh, cols] * inv[hh // 8][hh % 8:hh % 8 + 1, cols]
                                         for hh in range(H)], axis=0).astype(BF16)
                    fill = _Filler(z_v[...] != 0, 5 * D, steps)
                    for r in range(0, D, OR):
                        a = None
                        for k0, k1 in ((4 * L, D), (0, 2 * L), (2 * L, 4 * L)):
                            m = _dot(wot_v[r:r + OR, k0:k1], o[k0:k1])
                            fill.tick(m, OR * pl.cdiv(k1 - k0, L))
                            a = m if a is None else a + m
                        x1_v[r:r + OR, cols] = x_v[t, r:r + OR, cols].astype(F32) + mod(2, r, OR, 2) * a

                    def emit(r, norm, pair=pair):
                        h = [norm(r0) * mod(4, r0, 16, 2) + mod(3, r0, 16, 2) for r0 in (r, r + D // 2)]
                        for i, y in enumerate(_st_b([[hk[:, 0:L], hk[:, L:]] for hk in h])):
                            hb_v[i, r // 2:r // 2 + 8, pair * L:(pair + 1) * L] = _to_packed(y)
                    steps = _norm_steps(lambda r, n, cols=cols: x1_v[r:r + n, cols], D, emit, range(0, D // 2, 16))
                _run(steps)

            def gate_up(it):
                host = Host(t, it * HG, HG, UG * (47 * RB // 2 + 4 * sum(WT)))
                for uu in range(UG):
                    rows = pl.ds(pl.multiple_of((it * UG + uu) * (RB // 2), RB // 2), RB // 2)
                    sh = []
                    for i in range(7):
                        sh.append(_dot(_bc(ws_v[i, rows, :]), _bc(hb_v[i, 80:144, :])))
                        host.tick(sh[-1], RB // 2)
                    sh = _st_c(sh)
                    acts = []
                    for n in range(4):
                        ms = []
                        for i in range(7):
                            rhs = [hb_v[i, 0:64, :]] + [
                                hb_v[i, 64:80, :] if m == n else hb_v[i, 80 + 16 * m:96 + 16 * m, :] for m in range(4)]
                            ms.append(_dot(_bc(wa_v[i, n, rows, :]), _bc(jnp.concatenate(rhs, axis=0))))
                            host.tick(ms[-1], RB if i < 5 else WT[n % 2])
                        m1, m2, m3, m4, m5, m6, m7 = ms
                        acts.append([(g + g * jnp.tanh(g)) * u for g, u in (
                            (sh[0][0] + m1 + m4 - m5 + m7, sh[1][0] + m2 + m4),
                            (sh[0][1] + m3 + m5, sh[1][1] + m1 - m2 + m3 + m6))])
                        if n % 2 == 1:
                            for i, y in enumerate(_st_b(acts[n - 1:])):
                                ab_v[i, n // 2, pl.ds(pl.multiple_of((it * UG + uu) * RB, RB), RB), :] = y

            with scope("gateup"):
                loop(GI, gate_up)

            with scope("down"):
                host = Host(t, GI * HG, HD, 49 * NU * D // 16)
                mid = [None] * 7
                for i in (2, 4, 1, 3, 0, 6, 5):
                    ms = []
                    for k in range(7):
                        acc = None
                        for u0 in range(0, NU, 4):
                            u1 = min(u0 + 4, NU)
                            w = jnp.concatenate([wdc_v[7 * i + k, u] for u in range(u0, u1)], axis=1)
                            b = _st_b([[ab_v[i, r, u0 * L:u1 * L, c * L:(c + 1) * L] for c in range(2)]
                                       for r in range(2)])[k]
                            m = _dot(_bc(w), b.astype(BF16))
                            host.tick(m, (u1 - u0) * D // 16)
                            acc = m if acc is None else acc + m
                        ms.append(acc)
                    mid[i] = _st_c(ms)
                quad = [[_st_c([m[r][c] for m in mid]) for c in range(2)] for r in range(2)]
                y = jnp.concatenate([jnp.concatenate([quad[r % 2][c // 2][r // 2][c % 2] for c in range(4)], axis=1)
                                     for r in range(4)], axis=0)
                ob_v[t] = (x1_v[...] + mod(5, 0, D, 4) * y).astype(BF16)
                out_copy(t).start()

        loop(NQ, tile)
        for t in range(NQ):
            out_copy(t).wait()

    scratch = [
        pltpu.VMEM((NQ, D, TQ), BF16),
        pltpu.VMEM((D, D), BF16),
        pltpu.VMEM((D, D), BF16),
        pltpu.VMEM((3, 3, D, 4 * L), BF16),
        pltpu.VMEM((D, 6 * D), BF16),
        pltpu.VMEM((6, D, L), F32),
        pltpu.VMEM((2, D, TQ), BF16),
        pltpu.VMEM((3, 8, TQ), F32),
        pltpu.VMEM((32, L), F32),
        pltpu.VMEM((D + 64, D), BF16),
        pltpu.VMEM((D, D), BF16),
        pltpu.VMEM((NQ * NG, 4 * Dh, 3 * TQ), F32),
        pltpu.VMEM((S // 2, 32), U32),
        pltpu.VMEM((NB // 16, 66, 8, L), F32),
        pltpu.VMEM((NC, 24, L), F32),
        pltpu.VMEM((2, S // 2, TQ), U32),
        pltpu.VMEM((H, max(NH // 2, 8), TQ), U32),
        pltpu.VMEM((H, 24, TQ), F32),
        pltpu.VMEM((2, 2, 9, L // 2, L), U32),
        pltpu.VMEM((7, 4, NU * L // 2, 2 * L), U32),
        pltpu.VMEM((7, NU * L // 2, L), U32),
        pltpu.VMEM((52, NU, D // 8, L), U32),
        pltpu.VMEM((D, TQ), F32),
        pltpu.VMEM((7, D // 4, 2 * L), U32),
        pltpu.VMEM((7, 2, NU * L, 2 * L), F32),
        pltpu.VMEM((NQ, D, TQ), BF16),
        pltpu.VMEM((8, L), jnp.int32),
        pltpu.VMEM((Dh, D), BF16),
        pltpu.VMEM((Dh, D), BF16),
        pltpu.VMEM((1, D), BF16),
        pltpu.SemaphoreType.DMA((7,)),
        pltpu.SemaphoreType.DMA((NQ,)),
        pltpu.SemaphoreType.DMA((3, 3)),
        pltpu.SemaphoreType.DMA((NQ,)),
    ]
    return kernel, scratch


def build(**cfg):
    flags = cfg.pop("flags", None)

    def fn(A_x, A_wq, A_wk, A_wv, A_wo, B_x, B_w_gate, B_w_up, B_w_down, c, w_mod):
        _, S, D = A_x.shape
        F = B_w_gate.shape[1]
        kernel, scratch = make_kernel(S, D, F, **cfg)
        out_t = pl.pallas_call(
            kernel,
            in_specs=[pl.BlockSpec(memory_space=pl.ANY)] * 10,
            out_specs=pl.BlockSpec(memory_space=pl.ANY),
            out_shape=jax.ShapeDtypeStruct((D, S), A_x.dtype),
            scratch_shapes=scratch,
            compiler_params=pltpu.CompilerParams(vmem_limit_bytes=120 * 2 ** 20, flags=flags),
            name="adaln_block",
        )(A_x[0].T, A_wq, A_wk.T, A_wv.T, A_wo, B_w_gate, B_w_up, B_w_down.T, c, w_mod)
        return out_t.T[None]

    return fn


pallas_adaLN_cond__grouped_kv_mqa__swiglu_ffn__prompt_kernel = jax.jit(build())
```

```python
import functools
import math

import jax
import jax.numpy as jnp
from jax import lax
import jax.experimental.pallas as pl
import jax.experimental.pallas.tpu as pltpu

BF16, F32, U32 = jnp.bfloat16, jnp.float32, jnp.uint32
H = 32
EPS = 1e-5
L = 128
TQ = 4 * L
KB = 16
SAFE_SCORE = 60.0
SAFE_VALUE = 2.0 ** 50


def _dot(a, b):
    return jnp.dot(a, b, preferred_element_type=F32)


def _cat(xs, axis=0):
    return jnp.concatenate(xs, axis=axis)


def _words(x):
    return pltpu.bitcast(x.astype(BF16), U32)


def _all_words(xs):
    y = _words(_cat(xs, 1))
    return [y[:, n * L:(n + 1) * L] for n in range(len(xs))]


def _bf16(x):
    return pltpu.bitcast(x, BF16)


def _multiple(i, n):
    return pl.ds(pl.multiple_of(i * n, n), n)


def _strassen_lhs(a):
    (a11, a12), (a21, a22) = a
    return [a11 + a22, a21 + a22, a11, a22, a11 + a12, a21 - a11, a12 - a22]


def _strassen_rhs(b):
    (b11, b12), (b21, b22) = b
    return [b11 + b22, b11, b12 - b22, b21 - b11, b22, b11 + b12, b21 + b22]


def _strassen_add(c, i, m):
    for r, k, sign in (((0, 0, 1), (1, 1, 1)), ((1, 0, 1), (1, 1, -1)), ((0, 1, 1), (1, 1, 1)),
                       ((0, 0, 1), (1, 0, 1)), ((0, 0, -1), (0, 1, 1)), ((1, 1, 1),), ((0, 0, 1),))[i]:
        if c[r][k] is None:
            assert sign > 0
            c[r][k] = m
        else:
            c[r][k] = c[r][k] + m if sign > 0 else c[r][k] - m


def _swiglu(g, u):
    return (g + g * jnp.tanh(g)) * u


def _norm_steps(load, n, emit, rows):
    st = {}

    def fold(key, x):
        x = jnp.sum(x.reshape(-1, 8, x.shape[1]), axis=0)
        st[key] = st[key] + x if key in st else x

    def mean(key):
        return jnp.sum(st[key], axis=0, keepdims=True) * (1.0 / n)

    def sums(r, pin):
        fold("sum", load(r, 64))
        if r + 64 == n:
            st["mean"] = jnp.broadcast_to(mean("sum"), st["sum"].shape)

    def squares(r, pin):
        d = load(r, 64) - _cat([pin(st["mean"])] * 8)
        fold("sq", d * d)
        if r + 64 == n:
            st["rstd"] = lax.rsqrt(mean("sq") + EPS)

    def write(r, pin):
        mu = _cat([pin(st["mean"])] * 2)
        emit(r, lambda r0: (load(r0, 16) - mu) * st["rstd"])

    return ([functools.partial(sums, r) for r in range(0, n, 64)]
            + [functools.partial(squares, r) for r in range(0, n, 64)]
            + [functools.partial(write, r) for r in rows])


def _run(steps):
    for step in steps:
        step(lambda x: x)


class _Filler:
    def __init__(self, never, cycles, *streams):
        self.never = never
        self.now = 0
        due = [(e * cycles // len(st), n, e, step) for n, st in enumerate(streams) for e, step in enumerate(st)]
        self.due = sorted(due, key=lambda d: d[:3], reverse=True)

    def tick(self, result, cycles):
        while self.due and self.due[-1][0] < self.now + cycles:
            at, _, _, step = self.due.pop()
            r = 8 * ((at - self.now) * (result.shape[0] // 8) // cycles)
            step(functools.partial(self.pin, result[r:r + 8, 0:L]))
        self.now += cycles

    def pin(self, mark, x):
        tile = lambda a: _cat([_cat([a] * (x.shape[1] // L), 1)] * (x.shape[0] // 8))
        if x.dtype != mark.dtype:
            mark = pltpu.bitcast(mark, x.dtype)
        return jnp.where(tile(self.never), tile(mark), x)


def _loop(n, f):
    def body(i, carry):
        f(i)
        return carry
    lax.fori_loop(0, n, body, 0)


def _make_kernel(S, D, F):
    assert (S, D, F) == (2048, 576, 4608)
    Dh = D // H
    HALF = Dh // 2
    NQ = S // TQ
    NG = H // 4
    NC = S // L
    NU = F // (4 * L)
    RB, UG = 96, 6
    GI = NU * L // (RB * UG)
    NV0, NV1, NH_UP, NH_DOWN = 224, 352, 160, 64
    NH = NH_UP + NH_DOWN
    NB = (NQ + 1) * L
    scale = float(Dh ** -0.5 * math.log2(math.e))

    def kernel(x_hbm, wq_hbm, wk_hbm, wv_hbm, wo_hbm, wg_hbm, wu_hbm, wd_hbm, c_hbm, wm_hbm, out_hbm,
               x_v, x1_v, mod_v, norm_v, zero_v, wot_v, q_v, k_v, kb_v, v_v, s_v, o_v, wa_v, ws_v, wd_v):

        def filler(cycles, *streams):
            return _Filler(zero_v[0:8, :] != 0, cycles, *streams)

        def mod(i, r, n, tiles):
            return _cat([mod_v[i * D + r:i * D + r + n, :]] * tiles, 1)

        def square_dot(w_ref, a, order, fill):
            shared = _dot(_bf16(w_ref[:, 8 * L:9 * L]), a[4 * L - 64:D])
            fill.tick(shared, len(order) * D // 8)
            for l in order:
                cols = slice(l * L, (l + 1) * L)
                for half, rhs in enumerate((a[0:4 * L], _cat([a[0:4 * L - 64], a[4 * L:D]]))):
                    y = _dot(_bf16(w_ref[:, 4 * half * L:4 * (half + 1) * L]), rhs[:, cols])
                    fill.tick(y, D // 2)
                    yield l, half, y + shared[:, cols]

        def score_steps(i, j, b, store):
            st = {}
            q_at = [(0, 0), (HALF, 0), (HALF, 2), (0, 4), (0, 6), (0, 8), (0, 10)]
            n, ds = 2, 5

            def emit(keys, queries, s):
                for m in range(n):
                    store(KB * m + 8 * keys, slice(2 * queries * L, 2 * (queries + 1) * L), s[8 * m:8 * m + 8])

            def step(name, p, start, d0, pin):
                for d in range(d0, min(d0 + ds, HALF)):
                    r, l = j * Dh + q_at[p][0] + d, q_at[p][1]
                    k = _cat([kb_v[b + m, HALF * p + d] for m in range(n)])
                    q = _cat([jnp.broadcast_to(q_v[i, r:r + 1, m * L:(m + 1) * L], (8, L)) for m in (l, l + 1)], 1)
                    t = _cat([k, k], 1) * _cat([pin(q) if d == d0 else q] * n)
                    prev = name if d else start
                    st[name] = t if prev is None else st[prev] + t
                if d0 + ds < HALF:
                    return
                if name == "u1":
                    emit(0, 0, st[name])
                elif name == "u6":
                    emit(1, 0, st[name])
                elif name == "p5":
                    emit(1, 1, st["u3"] + st[name])
                    st["u4"] = st["u2"] + st[name]
                elif name == "u5":
                    emit(0, 1, st[name])
            plan = [("p1", 0, None), ("u1", 1, "p1"), ("u2", 5, "p1"), ("u3", 6, "u2"), ("u6", 3, "u3"),
                    ("p5", 4, None), ("u5", 2, "u4")]
            return [functools.partial(step, *p, d0) for p in plan for d0 in range(0, HALF, ds)]

        def weigh_values(slot, c, early, narrow=False):
            k0, k1, kh = c * L, (c + 1) * L, S - (0 if early is None else NH)
            parts = []
            if k0 < kh:
                parts.append(jnp.exp2(s_v[slot, k0:min(k1, kh), :]))
            if k1 > kh:
                parts.append(early[max(k0, kh) - kh:k1 - kh, :])
            p = _cat(parts)
            return _dot(v_v[c], p.astype(BF16) if early is None or narrow else p)

        def attend(i, nv, early, extra=()):
            nm = S - nv - (0 if early is None else NH)
            for j in range(4):
                q = _cat([q_v[i, j * Dh:(j + 1) * Dh, 0:TQ], jnp.zeros((32 - Dh, TQ), F32)]).astype(BF16)
                steps = []
                for k0 in range(nm, nm + nv, 2 * KB):
                    def store(r, cols, s, k0=k0):
                        s_v[j % 2, k0 + r:k0 + r + 8, cols] = s
                    steps += score_steps(i, j, (k0 - (S - NB)) // KB, store)
                fill = filler(nm + 24 * NC, steps, extra[j * len(extra) // 4:(j + 1) * len(extra) // 4])
                acc = None
                for c in range(NC):
                    lo, hi = 16 * (c * (nm // 16) // NC), 16 * ((c + 1) * (nm // 16) // NC)
                    s = _dot(_bf16(k_v[lo // 2:hi // 2, :]), q)
                    s_v[j % 2, lo:hi, :] = s
                    fill.tick(s, hi - lo)
                    o = weigh_values(1 - j % 2, c, None if early is None else early(j))
                    acc = o if acc is None else acc + o
                    fill.tick(o, 24)
                o_v[(4 * i + j + 2 * H - 1) % (2 * H)] = acc

        def attend_with_max(t, n):
            hh, cols = n // 4, _multiple(n % 4, L)
            q = q_v[t * NG + hh // 4, 0:Dh, cols]
            for j in range(1, 4):
                q = jnp.where(hh % 4 == j, q_v[t * NG + hh // 4, j * Dh:(j + 1) * Dh, cols], q)
            s = _dot(_bf16(k_v[...]), _cat([q, jnp.zeros((32 - Dh, L), F32)]).astype(BF16))
            p = jnp.exp2(s - jnp.max(s, axis=0, keepdims=True))
            o_v[t % 2 * H + hh, :, cols] = _dot(_cat([v_v[c] for c in range(NC)], 1), p)

        def first_phase(w_v, raw_v, wm_v, h_v, kx_v, wkv_v, wqt_v, wt_v, osem, xsems, wsems):
            cp_wo = pltpu.make_async_copy(wo_hbm, w_v.at[1], osem)

            def x_copy(t):
                return pltpu.make_async_copy(x_hbm.at[:, _multiple(t, TQ)], x_v.at[t], xsems.at[t])

            def unit_copies(u):
                cols = pl.ds(pl.multiple_of(2 * D + u * 2 * L, L), 2 * L)
                return [pltpu.make_async_copy(w.at[:, _multiple(u, 4 * L)], raw_v.at[u % 3, n], wsems.at[u % 3, n])
                        for n, w in enumerate((wg_hbm, wu_hbm, wd_hbm))] + [
                    pltpu.make_async_copy(wm_hbm.at[:, cols], wm_v.at[:, cols], wsems.at[u % 3, 3])]

            def modulation(at, n):
                m = _dot(wkv_v[48:64, :], wm_v[:, pl.ds(at, n)])[0:1]
                col = at + lax.broadcasted_iota(jnp.int32, (1, n), 1)
                within = lambda i: jnp.logical_and(col >= i * D, col < (i + 1) * D)
                m = jnp.where(jnp.logical_or(within(1), within(4)), m + 1.0, m)
                m = m * jnp.where(jnp.logical_or(within(3), within(4)), 0.5, jnp.where(within(5), 2.0, 1.0))
                mod_v[pl.ds(at, n), :] = jnp.broadcast_to(m, (L, n)).T

            def transposed(blk, pin):
                blk = _words(blk)
                head = _cat([pin(blk[0:8, 0:L]), blk[0:8, L:]], 1) if blk.shape[1] > L else pin(blk[0:8])
                return _words(_bf16(_cat([head, blk[8:]])).T)

            def square_steps(w_ref, dst):
                high = lax.broadcasted_iota(jnp.int32, (1, L), 1) >= 64
                minus = lambda a, b: _words(_bf16(a).astype(F32) - _bf16(jnp.where(high, b, 0)).astype(F32))

                def step(n, lo, hi, pin):
                    wt = transposed(_cat([w_ref[lo:lo + 64, :], w_ref[hi:hi + 64, :]]), pin)
                    top, bot = wt[0:D // 4], wt[D // 4:D // 2]
                    if n < 3:
                        dst[:, n * L:(n + 1) * L], dst[:, (n + 4) * L:(n + 5) * L] = top, bot
                    else:
                        dst[:, n * L:(n + 1) * L] = (
                            minus(top, bot) if n == 3 else minus(bot, top) if n == 7 else jnp.where(high, top, bot))
                tiles = [(n, n * L, n * L + 64) for n in range(4)] + [(7, 3 * L, 4 * L), (8, 4 * L - 64, 4 * L)]
                return [functools.partial(step, *t) for t in tiles]

            def key_steps(row, c, d, first=0):
                cols = {}

                def spread(e, pin):
                    rows = jnp.broadcast_to(row(d + e * HALF), (L, L))
                    cols[e] = _words(_cat([pin(rows[0:8]), rows[8:]]).astype(BF16).T)

                def combine(r, pin):
                    a1, a2 = [_bf16(pin(cols[e][8 * r:8 * r + 8])).astype(F32) for e in range(2)]
                    a11, a21, a12, a22 = a1[0:8], a1[8:16], a2[0:8], a2[8:16]
                    s1 = a21 + a22
                    s2 = s1 - a11
                    for p, a in enumerate((a11, a12, a12 - s2, -a22, s1, s2, a11 - a21)):
                        kb_v[8 * c + r, HALF * p + d] = a
                return ([functools.partial(spread, e) for e in range(2)],
                        [functools.partial(combine, r) for r in range(first, 8)])

            def project(t):
                @pl.when(t + 1 < NQ)
                def _():
                    x_copy(jnp.minimum(t + 1, NQ - 1)).wait()

                for at, copies in enumerate(([x_copy(2), x_copy(3)], [cp_wo] + unit_copies(0), unit_copies(1))):
                    @pl.when(t == at)
                    def _():
                        for cp in copies:
                            cp.start()

                @pl.when(t == NQ - 1)
                def _():
                    cp_wo.wait()

                h = h_v[t % 2]
                kv = _dot(wkv_v[0:48, :], h)
                k, v = kv[0:24] * scale, kv[24:48]
                for d in range(Dh):
                    kx_v[d, 0:1, :] = k[d:d + 1, TQ - 2 * L:TQ - L]
                keys = [key_steps(lambda d: k[d:d + 1, TQ - L:], t + 1, d) for d in range(HALF)]
                steps = [lambda pin: None] * 8 + keys[0][0]
                for d in range(HALF):
                    steps += (keys[d + 1][0] if d + 1 < HALF else []) + keys[d][1]

                def emit(r, norm):
                    h_v[(t + 1) % 2, r:r + 16, :] = (norm(r) * mod(1, r, 16, 4) + mod(0, r, 16, 4)).astype(BF16)
                nxt = jnp.minimum(t + 1, NQ - 1)
                fill = filler(9 * D // 2 - 100, steps, _norm_steps(
                    lambda r, n: x_v[nxt, r:r + n, :].astype(F32), D, emit, range(0, D, 16)),
                    square_steps(w_v.at[t // (NQ - 1)], wot_v))
                q2 = norm_v[0, 0:1, 0:L]
                low = {}
                for l, half, q in square_dot(wqt_v, h, (0, 2, 1, 3), fill):
                    up = _cat([q[HALF:], q[:HALF]])
                    parts = {l: q}
                    if l < 2:
                        low[half] = q, up
                    else:
                        t1 = q - low[half][0]
                        parts.update({l + 2: up - t1 - low[half][1], l + 4: t1, l + 6: up - t1, l + 8: up - q})
                    for m, y in parts.items():
                        q_v[pl.ds(t * NG + half * NG // 2, NG // 2), :, m * L:(m + 1) * L] = y.reshape(NG // 2, -1, L)
                    qq = q * q
                    for r in range(0, D // 2, Dh):
                        q2 = jnp.maximum(q2, jnp.sum(qq[r:r + Dh], axis=0, keepdims=True))
                norm_v[0, 0:1, 0:L] = q2
                norm_v[1, 0:1, :] = jnp.maximum(norm_v[1, 0:1, :], jnp.sum(k * k, axis=0, keepdims=True))
                norm_v[2, 0:1, :] = jnp.maximum(norm_v[2, 0:1, :], jnp.max(jnp.abs(v), axis=0, keepdims=True))
                kn = _words(_cat([k, jnp.zeros((L - 24, TQ), F32)]).astype(BF16).T)[:, 0:32]
                vn = jnp.where(lax.broadcasted_iota(jnp.int32, (24, TQ), 0) == Dh, 1.0, v)
                for c in range(4):
                    at = 3 * t + c if c < 3 else 3 * NQ + t
                    k_v[_multiple(at, L // 2), :] = kn[c * L // 2:(c + 1) * L // 2]
                    v_v[at] = vn[:, c * L:(c + 1) * L]

            def weight_steps(u):
                slot = u % 3
                lane = lax.broadcasted_iota(jnp.int32, (8, L), 1)

                def transpose(w, half, kind, pin):
                    rows = lambda r, m, n: raw_v[slot, w, pl.ds(half * D // 2 + r, m), n * L:(n + 1) * L]
                    if kind < 4:
                        blk = rows(0, L, kind)
                    elif kind < 8:
                        blk = _cat([rows(L if m == kind - 4 else 160 + 32 * m, 32, kind - 4) for m in range(4)])
                    else:
                        blk = _cat([rows(160 + 32 * m, 32, m) for m in range(4)])
                    wt_v[w, half, kind] = transposed(blk, pin)

                def combine(kind, r, pin):
                    block = lambda row, half, k: wt_v[r // 8 % 2, half, k, pl.ds(r // 16 * 16 + 8 * row, 8), :]

                    def operand(row, half):
                        x = _bf16(pin(block(row, half, kind))).astype(F32)
                        if 4 <= kind < 8:
                            x -= _bf16(jnp.where(lane // 32 == kind - 4, 0, block(row, half, 8))).astype(F32)
                        return x
                    rows = pl.ds(pl.multiple_of(u * (L // 2) + r, 8), 8)
                    y = _strassen_lhs([[operand(row, half) for half in range(2)] for row in range(2)])
                    if 4 <= kind < 8:
                        y = _all_words(y)
                    else:
                        y = _all_words(y[0:2] + y[4:7])
                        y[2:2] = [block(e, e, kind) for e in range(2)]
                    for i in range(7):
                        if kind == 8:
                            ws_v[i, rows, :] = y[i]
                        else:
                            wa_v[i, kind % 4, rows, kind // 4 * L:(kind // 4 + 1) * L] = y[i]

                outer = {}

                def down_outer(r, a, b, pin):
                    def operand(q, n):
                        x = raw_v[slot, 2, pl.ds(q * D // 4 + 2 * r, 16), n * L:(n + 1) * L]
                        return _bf16(pin(_words(x))).astype(F32)
                    outer[a, b] = _strassen_lhs([[operand(a + 2 * q, 2 * b + n) for n in range(2)] for q in range(2)])

                def down_inner(r, i, pin):
                    y = _words(_cat(_strassen_lhs([[pin(outer[a, b][i]) if a == b else outer[a, b][i]
                                                    for b in range(2)] for a in range(2)]), 1))
                    for k in range(7):
                        wd_v[7 * i + k, u, r:r + 8, :] = y[:, k * L:(k + 1) * L]

                steps = []
                kinds = [8, 0, 4, 1, 5, 2, 6, 3, 7]
                for n in range(10):
                    for e in range(8):
                        if n < 9 and e % 2 == 0:
                            steps.append(functools.partial(transpose, e // 4, e // 2 % 2, kinds[n]))
                        if n > 0:
                            steps.append(functools.partial(combine, kinds[n - 1], 8 * e))
                late = []
                for r in range(0, D // 8, 8):
                    late += [functools.partial(down_outer, r, a, b) for a in range(2) for b in range(2)]
                    late += [functools.partial(down_inner, r, i) for i in range(7)]
                mods = [lambda pin, n=n: modulation(pl.multiple_of(2 * D + (2 * u + n) * L, L), L) for n in range(2)]
                keys = key_steps(lambda d: kx_v[d, 0:1, :], 0, u, (NB - NV1 - NH) // KB)
                steps = steps[:20] + mods[:1] + steps[20:]
                late = keys[0] + late[:30] + keys[1] + late[30:60] + mods[1:] + late[60:]
                return steps + late + [lambda pin: None] * 4

            def prologue(wk_v, wv_v, c_v, sems):
                cp_c, cp_wq, cp_wk, cp_wv, cp_wm = [
                    pltpu.make_async_copy(src, dst, sems.at[n]) for n, (src, dst) in enumerate((
                        (c_hbm, c_v), (wq_hbm, w_v.at[0]), (wk_hbm, wk_v), (wv_hbm, wv_v),
                        (wm_hbm.at[:, pl.ds(0, 2 * D)], wm_v.at[:, pl.ds(0, 2 * D)])))]
                for cp in (cp_c, x_copy(0), cp_wm):
                    cp.start()
                zero_v[...] = jnp.zeros_like(zero_v)
                norm_v[...] = jnp.zeros_like(norm_v)
                s_v[1] = jnp.zeros(s_v.shape[1:], F32)
                x_copy(0).wait()
                for cp in (cp_wq, cp_wk, cp_wv):
                    cp.start()

                def keep(r, norm):
                    x1_v[r:r + 16, :] = norm(r)
                _run(_norm_steps(lambda r, n: x_v[0, r:r + n, :].astype(F32), D, keep, range(0, D, 16)))
                x_copy(1).start()
                cp_c.wait()
                cp_wm.wait()
                c = c_v[...].astype(F32)
                wkv_v[48:64, :] = jnp.broadcast_to(c * jax.nn.sigmoid(c), (16, D)).astype(BF16)
                modulation(0, 2 * D)
                h_v[0] = (x1_v[...] * mod(1, 0, D, 4) + mod(0, 0, D, 4)).astype(BF16)
                for cp in (cp_wq, cp_wk, cp_wv):
                    cp.wait()
                _run(square_steps(w_v.at[0], wqt_v))
                pad = jnp.zeros((24 - Dh, D), F32)
                wkv_v[0:48, :] = _cat([wk_v[...].astype(F32), pad, wv_v[...].astype(F32), pad]).astype(BF16)

            pl.run_scoped(prologue, pltpu.VMEM((Dh, D), BF16), pltpu.VMEM((Dh, D), BF16),
                          pltpu.VMEM((1, D), BF16), pltpu.SemaphoreType.DMA((5,)))
            _loop(NQ, project)

            def first_tile(u):
                for cp in unit_copies(u):
                    cp.wait()

                @pl.when(u + 2 < NU)
                def _():
                    for cp in unit_copies(jnp.minimum(u + 2, NU - 1)):
                        cp.start()
                attend(u, NV0, None, weight_steps(u))
            _loop(NU, first_tile)

        pl.run_scoped(
            first_phase,
            pltpu.VMEM((2, D, D), BF16), pltpu.VMEM((3, 3, D, 4 * L), BF16),
            pltpu.VMEM((D, 6 * D), BF16), pltpu.VMEM((2, D, TQ), BF16), pltpu.VMEM((Dh, 8, L), F32),
            pltpu.VMEM((64, D), BF16), pltpu.VMEM((D // 4, 9 * L), U32), pltpu.VMEM((2, 2, 9, L // 2, L), U32),
            pltpu.SemaphoreType.DMA(()), pltpu.SemaphoreType.DMA((NQ,)), pltpu.SemaphoreType.DMA((3, 4)))

        bound = jnp.max(norm_v[0, 0:1, :], axis=1, keepdims=True) * norm_v[1, 0:1, :]
        ok = jnp.logical_and(bound <= SAFE_SCORE ** 2, norm_v[2, 0:1, :] <= SAFE_VALUE)
        safe = jnp.max(jnp.where(ok, 0.0, 1.0)) < 0.5

        def second_phase(p_v, hb_v, act_v, out_v, sems):
            def out_copy(t, half):
                rows = pl.ds(half * D // 2, D // 2)
                return pltpu.make_async_copy(out_v.at[t, rows], out_hbm.at[rows, _multiple(t, TQ)], sems.at[t, half])

            def early_scores(t, first_head, heads, first_key, keys, cycles):
                steps = []
                for e in range(heads):
                    hh = first_head + e
                    for k0 in range(first_key, first_key + keys, 2 * KB):
                        def store(r, cols, s, k0=k0, hh=hh):
                            p_v[hh, k0 + r:k0 + r + 8, cols] = jnp.exp2(s)
                        steps += score_steps(jnp.minimum((t + 1) * NG + (hh + 3) // 4, NQ * NG - 1), (e + 3) % 4,
                                             (NB - NH + k0) // KB, store)
                return filler(cycles, steps)

            def project_heads(t):
                heads = o_v.at[pl.ds(t % 2 * H, H)]
                inv = [1.0 / heads[g:g + 8, Dh, :] for g in range(0, H, 8)]
                steps = []
                for pair in range(2):
                    cols = slice(2 * pair * L, 2 * (pair + 1) * L)
                    o = _cat([heads[hh, 0:Dh, cols] * inv[hh // 8][hh % 8:hh % 8 + 1, cols] for hh in range(H)])
                    for l, half, a in square_dot(wot_v, o.astype(BF16), (0, 1), filler(9 * D // 4, steps)):
                        r, c = half * D // 2, slice((2 * pair + l) * L, (2 * pair + l + 1) * L)
                        x1_v[r:r + D // 2, c] = x_v[t, r:r + D // 2, c].astype(F32) + mod(2, r, D // 2, 1) * a

                    def emit(r, norm, pair=pair):
                        h = [norm(r0) * mod(4, r0, 16, 2) + mod(3, r0, 16, 2) for r0 in (r, r + D // 2)]
                        y = _words(_cat(_strassen_rhs([[hk[:, 0:L], hk[:, L:]] for hk in h]), 1))
                        for i in range(7):
                            hb_v[i, r // 2:r // 2 + 8, pair * L:(pair + 1) * L] = y[:, i * L:(i + 1) * L]
                    steps = _norm_steps(lambda r, n, cols=cols: x1_v[r:r + n, cols], D, emit, range(0, D // 2, 16))
                _run(steps)

            def gate_up(t, it):
                room = ((96, 80, 96, 96, 80, 80, 80), (96, 60, 96, 96, 60, 60, 60))
                fill = early_scores(t, it * (H // GI), H // GI, 0, NH_UP, UG * (7 * 24 + 2 * sum(room[0] + room[1])))
                for block in range(UG):
                    rows = _multiple(it * UG + block, RB // 2)
                    shared = [[None] * 2 for _ in range(2)]
                    for i in range(7):
                        m = _dot(_bf16(ws_v[i, rows, :]), _bf16(hb_v[i, 80:144, :]))
                        fill.tick(m, 24)
                        _strassen_add(shared, i, m)
                    acts = []
                    for n in range(4):
                        c = [list(r) for r in shared]
                        for at, i in enumerate((2, 4, 0, 1, 5, 3, 6)):
                            rhs = [hb_v[i, 0:64, :]] + [
                                hb_v[i, pl.ds(64 if m == n else 80 + 16 * m, 16), :] for m in range(4)]
                            m = _dot(_bf16(wa_v[i, n, rows, :]), _bf16(_cat(rhs)))
                            fill.tick(m, room[n % 2][at])
                            _strassen_add(c, i, m)
                        acts.append([_cat([_swiglu(c[row][k][r:r + 16], c[row][k][r + 16:r + 32])
                                          for r in range(0, RB, 32) for row in range(2)]) for k in range(2)])
                        if n % 2 == 1:
                            for i, y in enumerate(_strassen_rhs(acts[n - 1:])):
                                act_v[i, n // 2, _multiple(it * UG + block, RB), :] = y

            def down(t):
                fill = early_scores(t, 0, H, NH_UP, NH_DOWN, 49 * NU * D // 16)
                y = [[[[None] * 2 for _ in range(2)] for _ in range(2)] for _ in range(2)]
                for i in (2, 3, 4, 1, 0, 6, 5):
                    c = [[None] * 2 for _ in range(2)]
                    for k in range(7):
                        acc = None
                        for u0, u1 in ((0, 4), (4, 5), (5, NU)):
                            b = _strassen_rhs([[act_v[i, r, u0 * L:u1 * L, n * L:(n + 1) * L] for n in range(2)]
                                               for r in range(2)])[k]
                            m = _dot(_bf16(_cat([wd_v[7 * i + k, u] for u in range(u0, u1)], 1)), b.astype(BF16))
                            fill.tick(m, (u1 - u0) * D // 16)
                            acc = m if acc is None else acc + m
                        _strassen_add(c, k, acc)
                    for r in range(2):
                        for n in range(2):
                            _strassen_add(y[r][n], i, c[r][n])
                    if i in (6, 5):
                        half = 6 - i
                        rows = slice(half * D // 2, (half + 1) * D // 2)
                        ffn = _cat([_cat([y[r][n // 2][half][n % 2] for n in range(4)], 1) for r in range(2)])
                        out_v[t, rows, :] = (x1_v[rows, :] + mod(5, rows.start, D // 2, 4) * ffn).astype(BF16)
                        out_copy(t, half).start()

            def tile(t):
                @pl.when(safe)
                def _():
                    _loop(jnp.where(t == 0, 0, jnp.where(t == NQ - 1, NG - 1, NG)),
                         lambda g: attend(t * NG + 1 + g, NV1, lambda j: p_v.at[4 * g + j]))

                    def last_head(_):
                        o_v[2 * H - 1] = sum(weigh_values(1, c, p_v.at[H - 4], True) for c in range(NC))
                    _loop(jnp.where(t == NQ - 1, 1, 0), last_head)

                @pl.when(jnp.logical_not(safe))
                def _():
                    _loop(4 * H, lambda n: attend_with_max(t, n))

                project_heads(t)
                _loop(GI, lambda it: gate_up(t, it))
                down(t)

            _loop(NQ, tile)
            for t in range(NQ):
                for half in range(2):
                    out_copy(t, half).wait()

        pl.run_scoped(
            second_phase,
            pltpu.VMEM((H, NH, TQ), F32), pltpu.VMEM((7, D // 4, 2 * L), U32),
            pltpu.VMEM((7, 2, NU * L, 2 * L), F32), pltpu.VMEM((NQ, D, TQ), BF16),
            pltpu.SemaphoreType.DMA((NQ, 2)))

    scratch = [
        pltpu.VMEM((NQ, D, TQ), BF16),
        pltpu.VMEM((D, TQ), F32),
        pltpu.VMEM((6 * D, L), F32),
        pltpu.VMEM((3, 8, TQ), F32),
        pltpu.VMEM((16, L), jnp.int32),
        pltpu.VMEM((D // 4, 9 * L), U32),
        pltpu.VMEM((NQ * NG, 4 * Dh, 3 * TQ), F32),
        pltpu.VMEM((S // 2, 32), U32),
        pltpu.VMEM((NB // KB, 66, 8, L), F32),
        pltpu.VMEM((NC, 24, L), F32),
        pltpu.VMEM((2, S, TQ), F32),
        pltpu.VMEM((2 * H, 24, TQ), F32),
        pltpu.VMEM((7, 4, NU * L // 2, 2 * L), U32),
        pltpu.VMEM((7, NU * L // 2, L), U32),
        pltpu.VMEM((51, NU, D // 8, L), U32),
    ]
    return kernel, scratch


@jax.jit
def pallas_adaLN_cond__grouped_kv_mqa__swiglu_ffn__prompt_kernel(
    A_x: jax.Array,
    A_wq: jax.Array,
    A_wk: jax.Array,
    A_wv: jax.Array,
    A_wo: jax.Array,
    B_x: jax.Array,
    B_w_gate: jax.Array,
    B_w_up: jax.Array,
    B_w_down: jax.Array,
    c: jax.Array,
    w_mod: jax.Array,
):
    del B_x
    _, S, D = A_x.shape
    kernel, scratch = _make_kernel(S, D, B_w_gate.shape[1])
    out_t = pl.pallas_call(
        kernel,
        in_specs=[pl.BlockSpec(memory_space=pl.ANY)] * 10,
        out_specs=pl.BlockSpec(memory_space=pl.ANY),
        out_shape=jax.ShapeDtypeStruct((D, S), A_x.dtype),
        scratch_shapes=scratch,
        compiler_params=pltpu.CompilerParams(vmem_limit_bytes=122 * 2 ** 20),
        name="adaln_block",
    )(A_x.reshape(S, D).T, A_wq, A_wk.T, A_wv.T, A_wo, B_w_gate, B_w_up, B_w_down.T, c, w_mod)
    return out_t.T.reshape(1, S, D)
```

```python
import functools
import math

import jax
import jax.numpy as jnp
from jax import lax
import jax.experimental.pallas as pl
import jax.experimental.pallas.tpu as pltpu

BF16, F32, U32 = jnp.bfloat16, jnp.float32, jnp.uint32
H = 32
EPS = 1e-5
L = 128
TQ = 4 * L
KB = 16
SAFE_SCORE = 60.0
SAFE_VALUE = 2.0 ** 50


def _dot(a, b):
    return jnp.dot(a, b, preferred_element_type=F32)


def _cat(xs, axis=0):
    return jnp.concatenate(xs, axis=axis)


def _words(x):
    return pltpu.bitcast(x.astype(BF16), U32)


def _all_words(xs):
    y = _words(_cat(xs, 1))
    return [y[:, n * L:(n + 1) * L] for n in range(len(xs))]


def _bf16(x):
    return pltpu.bitcast(x, BF16)


def _multiple(i, n):
    return pl.ds(pl.multiple_of(i * n, n), n)


def _strassen_lhs(a):
    (a11, a12), (a21, a22) = a
    return [a11 + a22, a21 + a22, a11, a22, a11 + a12, a21 - a11, a12 - a22]


def _strassen_rhs(b):
    (b11, b12), (b21, b22) = b
    return [b11 + b22, b11, b12 - b22, b21 - b11, b22, b11 + b12, b21 + b22]


def _strassen_add(c, i, m):
    for r, k, sign in (((0, 0, 1), (1, 1, 1)), ((1, 0, 1), (1, 1, -1)), ((0, 1, 1), (1, 1, 1)),
                       ((0, 0, 1), (1, 0, 1)), ((0, 0, -1), (0, 1, 1)), ((1, 1, 1),), ((0, 0, 1),))[i]:
        if c[r][k] is None:
            assert sign > 0
            c[r][k] = m
        else:
            c[r][k] = c[r][k] + m if sign > 0 else c[r][k] - m


def _swiglu(g, u):
    return (g + g * jnp.tanh(g)) * u


def _norm_steps(load, n, emit, rows):
    st = {}

    def fold(key, x):
        x = jnp.sum(x.reshape(-1, 8, x.shape[1]), axis=0)
        st[key] = st[key] + x if key in st else x

    def mean(key):
        return jnp.sum(st[key], axis=0, keepdims=True) * (1.0 / n)

    def sums(r, pin):
        fold("sum", load(r, 64))
        if r + 64 == n:
            st["mean"] = jnp.broadcast_to(mean("sum"), st["sum"].shape)

    def squares(r, pin):
        d = load(r, 64) - _cat([pin(st["mean"])] * 8)
        fold("sq", d * d)
        if r + 64 == n:
            st["rstd"] = lax.rsqrt(mean("sq") + EPS)

    def write(r, pin):
        mu = _cat([pin(st["mean"])] * 2)
        emit(r, lambda r0: (load(r0, 16) - mu) * st["rstd"])

    return ([functools.partial(sums, r) for r in range(0, n, 64)]
            + [functools.partial(squares, r) for r in range(0, n, 64)]
            + [functools.partial(write, r) for r in rows])


def _run(steps):
    for step in steps:
        step(lambda x: x)


class _Filler:
    def __init__(self, never, cycles, *streams):
        self.never = never
        self.now = 0
        due = [(e * cycles // len(st), n, e, step) for n, st in enumerate(streams) for e, step in enumerate(st)]
        self.due = sorted(due, key=lambda d: d[:3], reverse=True)

    def tick(self, result, cycles):
        while self.due and self.due[-1][0] < self.now + cycles:
            at, _, _, step = self.due.pop()
            r = 8 * ((at - self.now) * (result.shape[0] // 8) // cycles)
            step(functools.partial(self.pin, result[r:r + 8, 0:L]))
        self.now += cycles

    def pin(self, mark, x):
        tile = lambda a: _cat([_cat([a] * (x.shape[1] // L), 1)] * (x.shape[0] // 8))
        if x.dtype != mark.dtype:
            mark = pltpu.bitcast(mark, x.dtype)
        return jnp.where(tile(self.never), tile(mark), x)


def _loop(n, f):
    def body(i, carry):
        f(i)
        return carry
    lax.fori_loop(0, n, body, 0)


def _make_kernel(S, D, F):
    assert (S, D, F) == (2048, 576, 4608)
    Dh = D // H
    HALF = Dh // 2
    NQ = S // TQ
    NG = H // 4
    NC = S // L
    NU = F // (4 * L)
    RB, UG = 96, 6
    GI = NU * L // (RB * UG)
    NV0, NV1, NH_UP, NH_DOWN = 224, 352, 160, 64
    NH = NH_UP + NH_DOWN
    NB = (NQ + 1) * L
    scale = float(Dh ** -0.5 * math.log2(math.e))

    def kernel(x_hbm, wq_hbm, wk_hbm, wv_hbm, wo_hbm, wg_hbm, wu_hbm, wd_hbm, c_hbm, wm_hbm, out_hbm,
               x_v, x1_v, mod_v, norm_v, zero_v, wot_v, q_v, k_v, kb_v, v_v, s_v, o_v, wa_v, ws_v, wd_v):

        def filler(cycles, *streams):
            return _Filler(zero_v[0:8, :] != 0, cycles, *streams)

        def mod(i, r, n, tiles):
            return _cat([mod_v[i * D + r:i * D + r + n, :]] * tiles, 1)

        def square_dot(w_ref, a, order, fill):
            shared = _dot(_bf16(w_ref[:, 8 * L:9 * L]), a[4 * L - 64:D])
            fill.tick(shared, len(order) * D // 8)
            for l in order:
                cols = slice(l * L, (l + 1) * L)
                for half, rhs in enumerate((a[0:4 * L], _cat([a[0:4 * L - 64], a[4 * L:D]]))):
                    y = _dot(_bf16(w_ref[:, 4 * half * L:4 * (half + 1) * L]), rhs[:, cols])
                    fill.tick(y, D // 2)
                    yield l, half, y + shared[:, cols]

        def key_operand(b, e):
            k = _cat([kb_v[b, e], kb_v[b + 1, e]])
            return _cat([k, k], 1)

        def query_operand(i, j, r, l):
            r += j * Dh
            q = _cat([jnp.broadcast_to(q_v[i, r:r + 1, m * L:(m + 1) * L], (8, L)) for m in (l, l + 1)], 1)
            return q, _cat([q, q])

        def score_steps(keys, queries, b, store):
            st = {}
            q_at = [(0, 0), (HALF, 0), (HALF, 2), (0, 4), (0, 6), (0, 8), (0, 10)]
            ds = 5

            def emit(row, col, s):
                for m in range(2):
                    store(KB * m + 8 * row, slice(2 * col * L, 2 * (col + 1) * L), s[8 * m:8 * m + 8])

            def step(name, p, start, d0, pin):
                for d in range(d0, min(d0 + ds, HALF)):
                    k = keys(b, HALF * p + d)
                    q, qq = queries(q_at[p][0] + d, q_at[p][1])
                    t = k * (_cat([pin(q)] * 2) if d == d0 else qq)
                    prev = name if d else start
                    st[name] = t if prev is None else st[prev] + t
                if d0 + ds < HALF:
                    return
                if name == "u1":
                    emit(0, 0, st[name])
                elif name == "u6":
                    emit(1, 0, st[name])
                elif name == "p5":
                    emit(1, 1, st["u3"] + st[name])
                    st["u4"] = st["u2"] + st[name]
                elif name == "u5":
                    emit(0, 1, st[name])
            plan = [("p1", 0, None), ("u1", 1, "p1"), ("u2", 5, "p1"), ("u3", 6, "u2"), ("u6", 3, "u3"),
                    ("p5", 4, None), ("u5", 2, "u4")]
            return [functools.partial(step, *p, d0) for p in plan for d0 in range(0, HALF, ds)]

        def weigh_values(slot, c, early, narrow=False):
            k0, k1, kh = c * L, (c + 1) * L, S - (0 if early is None else NH)
            parts = []
            if k0 < kh:
                parts.append(jnp.exp2(s_v[slot, k0:min(k1, kh), :]))
            if k1 > kh:
                parts.append(early[max(k0, kh) - kh:k1 - kh, :])
            p = _cat(parts)
            return _dot(v_v[c], p.astype(BF16) if early is None or narrow else p)

        def attend(i, nv, early, extra=()):
            nm = S - nv - (0 if early is None else NH)
            keys = key_operand if extra else functools.cache(key_operand)
            for j in range(4):
                q = _cat([q_v[i, j * Dh:(j + 1) * Dh, 0:TQ], jnp.zeros((32 - Dh, TQ), F32)]).astype(BF16)
                steps, queries = [], functools.cache(functools.partial(query_operand, i, j))
                for k0 in range(nm, nm + nv, 2 * KB):
                    def store(r, cols, s, k0=k0):
                        s_v[j % 2, k0 + r:k0 + r + 8, cols] = s
                    steps += score_steps(keys, queries, (k0 - (S - NB)) // KB, store)
                fill = filler(nm + 24 * NC, steps, extra[j * len(extra) // 4:(j + 1) * len(extra) // 4])
                acc = None
                for c in range(NC):
                    lo, hi = 16 * (c * (nm // 16) // NC), 16 * ((c + 1) * (nm // 16) // NC)
                    s = _dot(_bf16(k_v[lo // 2:hi // 2, :]), q)
                    s_v[j % 2, lo:hi, :] = s
                    fill.tick(s, hi - lo)
                    o = weigh_values(1 - j % 2, c, None if early is None else early(j))
                    acc = o if acc is None else acc + o
                    fill.tick(o, 24)
                o_v[(4 * i + j + 2 * H - 1) % (2 * H)] = acc

        def attend_with_max(t, n):
            hh, cols = n // 4, _multiple(n % 4, L)
            q = q_v[t * NG + hh // 4, 0:Dh, cols]
            for j in range(1, 4):
                q = jnp.where(hh % 4 == j, q_v[t * NG + hh // 4, j * Dh:(j + 1) * Dh, cols], q)
            s = _dot(_bf16(k_v[...]), _cat([q, jnp.zeros((32 - Dh, L), F32)]).astype(BF16))
            p = jnp.exp2(s - jnp.max(s, axis=0, keepdims=True))
            o_v[t % 2 * H + hh, :, cols] = _dot(_cat([v_v[c] for c in range(NC)], 1), p)

        def first_phase(w_v, raw_v, wm_v, h_v, kx_v, wkv_v, wqt_v, wt_v, osem, xsems, wsems):
            cp_wo = pltpu.make_async_copy(wo_hbm, w_v.at[1], osem)

            def x_copy(t):
                return pltpu.make_async_copy(x_hbm.at[:, _multiple(t, TQ)], x_v.at[t], xsems.at[t])

            def unit_copies(u):
                cols = pl.ds(pl.multiple_of(2 * D + u * 2 * L, L), 2 * L)
                return [pltpu.make_async_copy(w.at[:, _multiple(u, 4 * L)], raw_v.at[u % 3, n], wsems.at[u % 3, n])
                        for n, w in enumerate((wg_hbm, wu_hbm, wd_hbm))] + [
                    pltpu.make_async_copy(wm_hbm.at[:, cols], wm_v.at[:, cols], wsems.at[u % 3, 3])]

            def modulation(at, n):
                m = _dot(wkv_v[48:64, :], wm_v[:, pl.ds(at, n)])[0:1]
                col = at + lax.broadcasted_iota(jnp.int32, (1, n), 1)
                within = lambda i: jnp.logical_and(col >= i * D, col < (i + 1) * D)
                m = jnp.where(jnp.logical_or(within(1), within(4)), m + 1.0, m)
                m = m * jnp.where(jnp.logical_or(within(3), within(4)), 0.5, jnp.where(within(5), 2.0, 1.0))
                mod_v[pl.ds(at, n), :] = jnp.broadcast_to(m, (L, n)).T

            def transposed(blk, pin):
                blk = _words(blk)
                head = _cat([pin(blk[0:8, 0:L]), blk[0:8, L:]], 1) if blk.shape[1] > L else pin(blk[0:8])
                return _words(_bf16(_cat([head, blk[8:]])).T)

            def square_steps(w_ref, dst):
                high = lax.broadcasted_iota(jnp.int32, (1, L), 1) >= 64
                minus = lambda a, b: _words(_bf16(a).astype(F32) - _bf16(jnp.where(high, b, 0)).astype(F32))

                def step(n, lo, hi, pin):
                    wt = transposed(_cat([w_ref[lo:lo + 64, :], w_ref[hi:hi + 64, :]]), pin)
                    top, bot = wt[0:D // 4], wt[D // 4:D // 2]
                    if n < 3:
                        dst[:, n * L:(n + 1) * L], dst[:, (n + 4) * L:(n + 5) * L] = top, bot
                    else:
                        dst[:, n * L:(n + 1) * L] = (
                            minus(top, bot) if n == 3 else minus(bot, top) if n == 7 else jnp.where(high, top, bot))
                tiles = [(n, n * L, n * L + 64) for n in range(4)] + [(7, 3 * L, 4 * L), (8, 4 * L - 64, 4 * L)]
                return [functools.partial(step, *t) for t in tiles]

            def key_steps(row, c, d, first=0):
                cols = {}

                def spread(e, pin):
                    rows = jnp.broadcast_to(row(d + e * HALF), (L, L))
                    cols[e] = _words(_cat([pin(rows[0:8]), rows[8:]]).astype(BF16).T)

                def combine(r, pin):
                    a1, a2 = [_bf16(pin(cols[e][8 * r:8 * r + 8])).astype(F32) for e in range(2)]
                    a11, a21, a12, a22 = a1[0:8], a1[8:16], a2[0:8], a2[8:16]
                    s1 = a21 + a22
                    s2 = s1 - a11
                    for p, a in enumerate((a11, a12, a12 - s2, -a22, s1, s2, a11 - a21)):
                        kb_v[8 * c + r, HALF * p + d] = a
                return ([functools.partial(spread, e) for e in range(2)],
                        [functools.partial(combine, r) for r in range(first, 8)])

            def project(t):
                @pl.when(t + 1 < NQ)
                def _():
                    x_copy(jnp.minimum(t + 1, NQ - 1)).wait()

                for at, copies in enumerate(([x_copy(2), x_copy(3)], [cp_wo] + unit_copies(0), unit_copies(1))):
                    @pl.when(t == at)
                    def _():
                        for cp in copies:
                            cp.start()

                @pl.when(t == NQ - 1)
                def _():
                    cp_wo.wait()

                h = h_v[t % 2]
                kv = _dot(wkv_v[0:48, :], h)
                k, v = kv[0:24] * scale, kv[24:48]
                for d in range(Dh):
                    kx_v[d, 0:1, :] = k[d:d + 1, TQ - 2 * L:TQ - L]
                keys = [key_steps(lambda d: k[d:d + 1, TQ - L:], t + 1, d) for d in range(HALF)]
                steps = [lambda pin: None] * 8 + keys[0][0]
                for d in range(HALF):
                    steps += (keys[d + 1][0] if d + 1 < HALF else []) + keys[d][1]

                def emit(r, norm):
                    h_v[(t + 1) % 2, r:r + 16, :] = (norm(r) * mod(1, r, 16, 4) + mod(0, r, 16, 4)).astype(BF16)
                nxt = jnp.minimum(t + 1, NQ - 1)
                fill = filler(9 * D // 2 - 100, steps, _norm_steps(
                    lambda r, n: x_v[nxt, r:r + n, :].astype(F32), D, emit, range(0, D, 16)),
                    square_steps(w_v.at[t // (NQ - 1)], wot_v))
                q2 = norm_v[0, 0:1, 0:L]
                low = {}
                for l, half, q in square_dot(wqt_v, h, (0, 2, 1, 3), fill):
                    up = _cat([q[HALF:], q[:HALF]])
                    parts = {l: q}
                    if l < 2:
                        low[half] = q, up
                    else:
                        t1 = q - low[half][0]
                        parts.update({l + 2: up - t1 - low[half][1], l + 4: t1, l + 6: up - t1, l + 8: up - q})
                    for m, y in parts.items():
                        q_v[pl.ds(t * NG + half * NG // 2, NG // 2), :, m * L:(m + 1) * L] = y.reshape(NG // 2, -1, L)
                    qq = q * q
                    for r in range(0, D // 2, Dh):
                        q2 = jnp.maximum(q2, jnp.sum(qq[r:r + Dh], axis=0, keepdims=True))
                norm_v[0, 0:1, 0:L] = q2
                norm_v[1, 0:1, :] = jnp.maximum(norm_v[1, 0:1, :], jnp.sum(k * k, axis=0, keepdims=True))
                norm_v[2, 0:1, :] = jnp.maximum(norm_v[2, 0:1, :], jnp.max(jnp.abs(v), axis=0, keepdims=True))
                kn = _words(_cat([k, jnp.zeros((L - 24, TQ), F32)]).astype(BF16).T)[:, 0:32]
                vn = jnp.where(lax.broadcasted_iota(jnp.int32, (24, TQ), 0) == Dh, 1.0, v)
                for c in range(4):
                    at = 3 * t + c if c < 3 else 3 * NQ + t
                    k_v[_multiple(at, L // 2), :] = kn[c * L // 2:(c + 1) * L // 2]
                    v_v[at] = vn[:, c * L:(c + 1) * L]

            def weight_steps(u):
                slot = u % 3
                lane = lax.broadcasted_iota(jnp.int32, (8, L), 1)

                def transpose(w, half, kind, pin):
                    rows = lambda r, m, n: raw_v[slot, w, pl.ds(half * D // 2 + r, m), n * L:(n + 1) * L]
                    if kind < 4:
                        blk = rows(0, L, kind)
                    elif kind < 8:
                        blk = _cat([rows(L if m == kind - 4 else 160 + 32 * m, 32, kind - 4) for m in range(4)])
                    else:
                        blk = _cat([rows(160 + 32 * m, 32, m) for m in range(4)])
                    wt_v[w, half, kind] = transposed(blk, pin)

                def combine(kind, r, pin):
                    block = lambda row, half, k: wt_v[r // 8 % 2, half, k, pl.ds(r // 16 * 16 + 8 * row, 8), :]

                    def operand(row, half):
                        x = _bf16(pin(block(row, half, kind))).astype(F32)
                        if 4 <= kind < 8:
                            x -= _bf16(jnp.where(lane // 32 == kind - 4, 0, block(row, half, 8))).astype(F32)
                        return x
                    rows = pl.ds(pl.multiple_of(u * (L // 2) + r, 8), 8)
                    y = _strassen_lhs([[operand(row, half) for half in range(2)] for row in range(2)])
                    if 4 <= kind < 8:
                        y = _all_words(y)
                    else:
                        y = _all_words(y[0:2] + y[4:7])
                        y[2:2] = [block(e, e, kind) for e in range(2)]
                    for i in range(7):
                        if kind == 8:
                            ws_v[i, rows, :] = y[i]
                        else:
                            wa_v[i, kind % 4, rows, kind // 4 * L:(kind // 4 + 1) * L] = y[i]

                outer = {}

                def down_outer(r, a, b, pin):
                    def operand(q, n):
                        x = raw_v[slot, 2, pl.ds(q * D // 4 + 2 * r, 16), n * L:(n + 1) * L]
                        return _bf16(pin(_words(x))).astype(F32)
                    outer[a, b] = _strassen_lhs([[operand(a + 2 * q, 2 * b + n) for n in range(2)] for q in range(2)])

                def down_inner(r, i, pin):
                    y = _words(_cat(_strassen_lhs([[pin(outer[a, b][i]) if a == b else outer[a, b][i]
                                                    for b in range(2)] for a in range(2)]), 1))
                    for k in range(7):
                        wd_v[7 * i + k, u, r:r + 8, :] = y[:, k * L:(k + 1) * L]

                steps = []
                kinds = [8, 0, 4, 1, 5, 2, 6, 3, 7]
                for n in range(10):
                    for e in range(8):
                        if n < 9 and e % 2 == 0:
                            steps.append(functools.partial(transpose, e // 4, e // 2 % 2, kinds[n]))
                        if n > 0:
                            steps.append(functools.partial(combine, kinds[n - 1], 8 * e))
                late = []
                for r in range(0, D // 8, 8):
                    late += [functools.partial(down_outer, r, a, b) for a in range(2) for b in range(2)]
                    late += [functools.partial(down_inner, r, i) for i in range(7)]
                mods = [lambda pin, n=n: modulation(pl.multiple_of(2 * D + (2 * u + n) * L, L), L) for n in range(2)]
                keys = key_steps(lambda d: kx_v[d, 0:1, :], 0, u, (NB - NV1 - NH) // KB)
                steps = steps[:20] + mods[:1] + steps[20:]
                late = keys[0] + late[:30] + keys[1] + late[30:60] + mods[1:] + late[60:]
                return steps + late + [lambda pin: None] * 4

            def prologue(wk_v, wv_v, c_v, sems):
                cp_c, cp_wq, cp_wk, cp_wv, cp_wm = [
                    pltpu.make_async_copy(src, dst, sems.at[n]) for n, (src, dst) in enumerate((
                        (c_hbm, c_v), (wq_hbm, w_v.at[0]), (wk_hbm, wk_v), (wv_hbm, wv_v),
                        (wm_hbm.at[:, pl.ds(0, 2 * D)], wm_v.at[:, pl.ds(0, 2 * D)])))]
                for cp in (cp_c, x_copy(0), cp_wm):
                    cp.start()
                zero_v[...] = jnp.zeros_like(zero_v)
                norm_v[...] = jnp.zeros_like(norm_v)
                s_v[1] = jnp.zeros(s_v.shape[1:], F32)
                x_copy(0).wait()
                for cp in (cp_wq, cp_wk, cp_wv):
                    cp.start()

                def keep(r, norm):
                    x1_v[r:r + 16, :] = norm(r)
                _run(_norm_steps(lambda r, n: x_v[0, r:r + n, :].astype(F32), D, keep, range(0, D, 16)))
                x_copy(1).start()
                cp_c.wait()
                cp_wm.wait()
                c = c_v[...].astype(F32)
                wkv_v[48:64, :] = jnp.broadcast_to(c * jax.nn.sigmoid(c), (16, D)).astype(BF16)
                modulation(0, 2 * D)
                h_v[0] = (x1_v[...] * mod(1, 0, D, 4) + mod(0, 0, D, 4)).astype(BF16)
                for cp in (cp_wq, cp_wk, cp_wv):
                    cp.wait()
                _run(square_steps(w_v.at[0], wqt_v))
                pad = jnp.zeros((24 - Dh, D), F32)
                wkv_v[0:48, :] = _cat([wk_v[...].astype(F32), pad, wv_v[...].astype(F32), pad]).astype(BF16)

            pl.run_scoped(prologue, pltpu.VMEM((Dh, D), BF16), pltpu.VMEM((Dh, D), BF16),
                          pltpu.VMEM((1, D), BF16), pltpu.SemaphoreType.DMA((5,)))
            _loop(NQ, project)

            def first_tile(u):
                for cp in unit_copies(u):
                    cp.wait()

                @pl.when(u + 2 < NU)
                def _():
                    for cp in unit_copies(jnp.minimum(u + 2, NU - 1)):
                        cp.start()
                attend(u, NV0, None, weight_steps(u))
            _loop(NU, first_tile)

        pl.run_scoped(
            first_phase,
            pltpu.VMEM((2, D, D), BF16), pltpu.VMEM((3, 3, D, 4 * L), BF16),
            pltpu.VMEM((D, 6 * D), BF16), pltpu.VMEM((2, D, TQ), BF16), pltpu.VMEM((Dh, 8, L), F32),
            pltpu.VMEM((64, D), BF16), pltpu.VMEM((D // 4, 9 * L), U32), pltpu.VMEM((2, 2, 9, L // 2, L), U32),
            pltpu.SemaphoreType.DMA(()), pltpu.SemaphoreType.DMA((NQ,)), pltpu.SemaphoreType.DMA((3, 4)))

        bound = jnp.max(norm_v[0, 0:1, :], axis=1, keepdims=True) * norm_v[1, 0:1, :]
        ok = jnp.logical_and(bound <= SAFE_SCORE ** 2, norm_v[2, 0:1, :] <= SAFE_VALUE)
        safe = jnp.max(jnp.where(ok, 0.0, 1.0)) < 0.5

        def second_phase(p_v, hb_v, act_v, out_v, sems):
            def out_copy(t, half):
                rows = pl.ds(half * D // 2, D // 2)
                return pltpu.make_async_copy(out_v.at[t, rows], out_hbm.at[rows, _multiple(t, TQ)], sems.at[t, half])

            def early_scores(t, reuse, first_head, heads, first_key, keys, cycles):
                steps, operands = [], reuse(key_operand)
                for e in range(heads):
                    hh = first_head + e
                    queries = reuse(functools.partial(
                        query_operand, jnp.minimum((t + 1) * NG + (hh + 3) // 4, NQ * NG - 1), (e + 3) % 4))
                    for k0 in range(first_key, first_key + keys, 2 * KB):
                        def store(r, cols, s, k0=k0, hh=hh):
                            p_v[hh, k0 + r:k0 + r + 8, cols] = jnp.exp2(s)
                        steps += score_steps(operands, queries, (NB - NH + k0) // KB, store)
                return filler(cycles, steps)

            def project_heads(t):
                heads = o_v.at[pl.ds(t % 2 * H, H)]
                inv = [1.0 / heads[g:g + 8, Dh, :] for g in range(0, H, 8)]
                steps = []
                for pair in range(2):
                    cols = slice(2 * pair * L, 2 * (pair + 1) * L)
                    o = _cat([heads[hh, 0:Dh, cols] * inv[hh // 8][hh % 8:hh % 8 + 1, cols] for hh in range(H)])
                    for l, half, a in square_dot(wot_v, o.astype(BF16), (0, 1), filler(9 * D // 4, steps)):
                        r, c = half * D // 2, slice((2 * pair + l) * L, (2 * pair + l + 1) * L)
                        x1_v[r:r + D // 2, c] = x_v[t, r:r + D // 2, c].astype(F32) + mod(2, r, D // 2, 1) * a

                    def emit(r, norm, pair=pair):
                        h = [norm(r0) * mod(4, r0, 16, 2) + mod(3, r0, 16, 2) for r0 in (r, r + D // 2)]
                        y = _words(_cat(_strassen_rhs([[hk[:, 0:L], hk[:, L:]] for hk in h]), 1))
                        for i in range(7):
                            hb_v[i, r // 2:r // 2 + 8, pair * L:(pair + 1) * L] = y[:, i * L:(i + 1) * L]
                    steps = _norm_steps(lambda r, n, cols=cols: x1_v[r:r + n, cols], D, emit, range(0, D // 2, 16))
                _run(steps)

            def gate_up(t, it):
                room = ((96, 80, 96, 96, 80, 80, 80), (96, 60, 96, 96, 60, 60, 60))
                fill = early_scores(t, functools.cache, it * (H // GI), H // GI, 0, NH_UP,
                                    UG * (7 * 24 + 2 * sum(room[0] + room[1])))
                for block in range(UG):
                    rows = _multiple(it * UG + block, RB // 2)
                    shared = [[None] * 2 for _ in range(2)]
                    for i in range(7):
                        m = _dot(_bf16(ws_v[i, rows, :]), _bf16(hb_v[i, 80:144, :]))
                        fill.tick(m, 24)
                        _strassen_add(shared, i, m)
                    acts = []
                    for n in range(4):
                        c = [list(r) for r in shared]
                        for at, i in enumerate((2, 4, 0, 1, 5, 3, 6)):
                            rhs = [hb_v[i, 0:64, :]] + [
                                hb_v[i, pl.ds(64 if m == n else 80 + 16 * m, 16), :] for m in range(4)]
                            m = _dot(_bf16(wa_v[i, n, rows, :]), _bf16(_cat(rhs)))
                            fill.tick(m, room[n % 2][at])
                            _strassen_add(c, i, m)
                        acts.append([_cat([_swiglu(c[row][k][r:r + 16], c[row][k][r + 16:r + 32])
                                          for r in range(0, RB, 32) for row in range(2)]) for k in range(2)])
                        if n % 2 == 1:
                            for i, y in enumerate(_strassen_rhs(acts[n - 1:])):
                                act_v[i, n // 2, _multiple(it * UG + block, RB), :] = y

            def down(t):
                fill = early_scores(t, lambda f: f, 0, H, NH_UP, NH_DOWN, 49 * NU * D // 16)
                y = [[[[None] * 2 for _ in range(2)] for _ in range(2)] for _ in range(2)]
                for i in (2, 3, 4, 1, 0, 6, 5):
                    c = [[None] * 2 for _ in range(2)]
                    for k in range(7):
                        acc = None
                        for u0, u1 in ((0, 4), (4, 5), (5, NU)):
                            b = _strassen_rhs([[act_v[i, r, u0 * L:u1 * L, n * L:(n + 1) * L] for n in range(2)]
                                               for r in range(2)])[k]
                            m = _dot(_bf16(_cat([wd_v[7 * i + k, u] for u in range(u0, u1)], 1)), b.astype(BF16))
                            fill.tick(m, (u1 - u0) * D // 16)
                            acc = m if acc is None else acc + m
                        _strassen_add(c, k, acc)
                    for r in range(2):
                        for n in range(2):
                            _strassen_add(y[r][n], i, c[r][n])
                    if i in (6, 5):
                        half = 6 - i
                        rows = slice(half * D // 2, (half + 1) * D // 2)
                        ffn = _cat([_cat([y[r][n // 2][half][n % 2] for n in range(4)], 1) for r in range(2)])
                        out_v[t, rows, :] = (x1_v[rows, :] + mod(5, rows.start, D // 2, 4) * ffn).astype(BF16)
                        out_copy(t, half).start()

            def tile(t):
                @pl.when(safe)
                def _():
                    _loop(jnp.where(t == 0, 0, jnp.where(t == NQ - 1, NG - 1, NG)),
                          lambda g: attend(t * NG + 1 + g, NV1, lambda j: p_v.at[4 * g + j]))

                    def last_head(_):
                        o_v[2 * H - 1] = sum(weigh_values(1, c, p_v.at[H - 4], True) for c in range(NC))
                    _loop(jnp.where(t == NQ - 1, 1, 0), last_head)

                @pl.when(jnp.logical_not(safe))
                def _():
                    _loop(4 * H, lambda n: attend_with_max(t, n))

                project_heads(t)
                _loop(GI, lambda it: gate_up(t, it))
                down(t)

            _loop(NQ, tile)
            for t in range(NQ):
                for half in range(2):
                    out_copy(t, half).wait()

        pl.run_scoped(
            second_phase,
            pltpu.VMEM((H, NH, TQ), F32), pltpu.VMEM((7, D // 4, 2 * L), U32),
            pltpu.VMEM((7, 2, NU * L, 2 * L), F32), pltpu.VMEM((NQ, D, TQ), BF16),
            pltpu.SemaphoreType.DMA((NQ, 2)))

    scratch = [
        pltpu.VMEM((NQ, D, TQ), BF16),
        pltpu.VMEM((D, TQ), F32),
        pltpu.VMEM((6 * D, L), F32),
        pltpu.VMEM((3, 8, TQ), F32),
        pltpu.VMEM((16, L), jnp.int32),
        pltpu.VMEM((D // 4, 9 * L), U32),
        pltpu.VMEM((NQ * NG, 4 * Dh, 3 * TQ), F32),
        pltpu.VMEM((S // 2, 32), U32),
        pltpu.VMEM((NB // KB, 66, 8, L), F32),
        pltpu.VMEM((NC, 24, L), F32),
        pltpu.VMEM((2, S, TQ), F32),
        pltpu.VMEM((2 * H, 24, TQ), F32),
        pltpu.VMEM((7, 4, NU * L // 2, 2 * L), U32),
        pltpu.VMEM((7, NU * L // 2, L), U32),
        pltpu.VMEM((51, NU, D // 8, L), U32),
    ]
    return kernel, scratch


@jax.jit
def pallas_adaLN_cond__grouped_kv_mqa__swiglu_ffn__prompt_kernel(
    A_x: jax.Array,
    A_wq: jax.Array,
    A_wk: jax.Array,
    A_wv: jax.Array,
    A_wo: jax.Array,
    B_x: jax.Array,
    B_w_gate: jax.Array,
    B_w_up: jax.Array,
    B_w_down: jax.Array,
    c: jax.Array,
    w_mod: jax.Array,
):
    del B_x
    _, S, D = A_x.shape
    kernel, scratch = _make_kernel(S, D, B_w_gate.shape[1])
    out_t = pl.pallas_call(
        kernel,
        in_specs=[pl.BlockSpec(memory_space=pl.ANY)] * 10,
        out_specs=pl.BlockSpec(memory_space=pl.ANY),
        out_shape=jax.ShapeDtypeStruct((D, S), A_x.dtype),
        scratch_shapes=scratch,
        compiler_params=pltpu.CompilerParams(vmem_limit_bytes=122 * 2 ** 20),
        name="adaln_block",
    )(A_x.reshape(S, D).T, A_wq, A_wk.T, A_wv.T, A_wo, B_w_gate, B_w_up, B_w_down.T, c, w_mod)
    return out_t.T.reshape(1, S, D)
```

```python
import functools
import math

import jax
import jax.numpy as jnp
from jax import lax
import jax.experimental.pallas as pl
import jax.experimental.pallas.tpu as pltpu

BF16, F32, U32 = jnp.bfloat16, jnp.float32, jnp.uint32
H = 32
EPS = 1e-5
L = 128
TQ = 4 * L
KB = 16
SAFE_SCORE = 60.0
SAFE_VALUE = 2.0 ** 50


def _dot(a, b):
    return jnp.dot(a, b, preferred_element_type=F32)


def _cat(xs, axis=0):
    return jnp.concatenate(xs, axis=axis)


def _words(x):
    return pltpu.bitcast(x.astype(BF16), U32)


def _all_words(xs):
    y = _words(_cat(xs, 1))
    return [y[:, n * L:(n + 1) * L] for n in range(len(xs))]


def _bf16(x):
    return pltpu.bitcast(x, BF16)


def _multiple(i, n):
    return pl.ds(pl.multiple_of(i * n, n), n)


def _strassen_lhs(a):
    (a11, a12), (a21, a22) = a
    return [a11 + a22, a21 + a22, a11, a22, a11 + a12, a21 - a11, a12 - a22]


def _strassen_rhs(b):
    (b11, b12), (b21, b22) = b
    return [b11 + b22, b11, b12 - b22, b21 - b11, b22, b11 + b12, b21 + b22]


def _strassen_add(c, i, m):
    for r, k, sign in (((0, 0, 1), (1, 1, 1)), ((1, 0, 1), (1, 1, -1)), ((0, 1, 1), (1, 1, 1)),
                       ((0, 0, 1), (1, 0, 1)), ((0, 0, -1), (0, 1, 1)), ((1, 1, 1),), ((0, 0, 1),))[i]:
        if c[r][k] is None:
            assert sign > 0
            c[r][k] = m
        else:
            c[r][k] = c[r][k] + m if sign > 0 else c[r][k] - m


def _swiglu(g, u):
    return (g + g * jnp.tanh(g)) * u


def _norm_steps(load, n, emit, rows):
    st = {}

    def fold(key, x):
        x = jnp.sum(x.reshape(-1, 8, x.shape[1]), axis=0)
        st[key] = st[key] + x if key in st else x

    def mean(key):
        return jnp.sum(st[key], axis=0, keepdims=True) * (1.0 / n)

    def sums(r, pin):
        fold("sum", load(r, 64))
        if r + 64 == n:
            st["mean"] = jnp.broadcast_to(mean("sum"), st["sum"].shape)

    def squares(r, pin):
        d = load(r, 64) - _cat([pin(st["mean"])] * 8)
        fold("sq", d * d)
        if r + 64 == n:
            st["rstd"] = lax.rsqrt(mean("sq") + EPS)

    def write(r, pin):
        mu = _cat([pin(st["mean"])] * 2)
        emit(r, lambda r0: (load(r0, 16) - mu) * st["rstd"])

    return ([functools.partial(sums, r) for r in range(0, n, 64)]
            + [functools.partial(squares, r) for r in range(0, n, 64)]
            + [functools.partial(write, r) for r in rows])


def _run(steps):
    for step in steps:
        step(lambda x: x)


class _Filler:
    def __init__(self, never, cycles, *streams):
        self.never = never
        self.now = 0
        due = [(e * cycles // len(st), n, e, step) for n, st in enumerate(streams) for e, step in enumerate(st)]
        self.due = sorted(due, key=lambda d: d[:3], reverse=True)

    def tick(self, result, cycles):
        while self.due and self.due[-1][0] < self.now + cycles:
            at, _, _, step = self.due.pop()
            r = 8 * ((at - self.now) * (result.shape[0] // 8) // cycles)
            step(functools.partial(self.pin, result[r:r + 8, 0:L]))
        self.now += cycles

    def pin(self, mark, x):
        tile = lambda a: _cat([_cat([a] * (x.shape[1] // L), 1)] * (x.shape[0] // 8))
        if x.dtype != mark.dtype:
            mark = pltpu.bitcast(mark, x.dtype)
        return jnp.where(tile(self.never), tile(mark), x)


def _loop(n, f):
    def body(i, carry):
        f(i)
        return carry
    lax.fori_loop(0, n, body, 0)


def _make_kernel(S, D, F):
    assert (S, D, F) == (2048, 576, 4608)
    Dh = D // H
    HALF = Dh // 2
    NQ = S // TQ
    NG = H // 4
    NC = S // L
    NU = F // (4 * L)
    RB, UG = 96, 6
    GI = NU * L // (RB * UG)
    NV0, NV1, NH_UP, NH_DOWN = 224, 352, 160, 64
    NH = NH_UP + NH_DOWN
    NB = (NQ + 1) * L
    scale = float(Dh ** -0.5 * math.log2(math.e))

    def kernel(x_hbm, wq_hbm, wk_hbm, wv_hbm, wo_hbm, wg_hbm, wu_hbm, wd_hbm, c_hbm, wm_hbm, out_hbm,
               x_v, x1_v, mod_v, norm_v, zero_v, wot_v, q_v, k_v, kb_v, v_v, s_v, o_v, wa_v, ws_v, wd_v):

        def filler(cycles, *streams):
            return _Filler(zero_v[0:8, :] != 0, cycles, *streams)

        def mod(i, r, n, tiles):
            return _cat([mod_v[i * D + r:i * D + r + n, :]] * tiles, 1)

        def square_dot(w_ref, a, order, fill):
            shared = _dot(_bf16(w_ref[:, 8 * L:9 * L]), a[4 * L - 64:D])
            fill.tick(shared, len(order) * D // 8)
            for l in order:
                cols = slice(l * L, (l + 1) * L)
                for half, rhs in enumerate((a[0:4 * L], _cat([a[0:4 * L - 64], a[4 * L:D]]))):
                    y = _dot(_bf16(w_ref[:, 4 * half * L:4 * (half + 1) * L]), rhs[:, cols])
                    fill.tick(y, D // 2)
                    yield l, half, y + shared[:, cols]

        def key_operand(b, e):
            k = _cat([kb_v[b, e], kb_v[b + 1, e]])
            return _cat([k, k], 1)

        def query_operand(i, j, r, l):
            r += j * Dh
            q = _cat([jnp.broadcast_to(q_v[i, r:r + 1, m * L:(m + 1) * L], (8, L)) for m in (l, l + 1)], 1)
            return q, _cat([q, q])

        def score_steps(keys, queries, b, store, p5_first=False):
            st = {}
            q_at = [(0, 0), (HALF, 0), (HALF, 2), (0, 4), (0, 6), (0, 8), (0, 10)]
            ds = 5

            def emit(row, col, s):
                for m in range(2):
                    store(KB * m + 8 * row, slice(2 * col * L, 2 * (col + 1) * L), s[8 * m:8 * m + 8])

            def step(name, p, start, d0, pin):
                for d in range(d0, min(d0 + ds, HALF)):
                    k = keys(b, HALF * p + d)
                    q, qq = queries(q_at[p][0] + d, q_at[p][1])
                    t = k * (_cat([pin(q)] * 2) if d == d0 else qq)
                    prev = name if d else start
                    st[name] = t if prev is None else st[prev] + t
                if d0 + ds < HALF:
                    return
                if name == "u1":
                    emit(0, 0, st[name])
                elif name == "u6":
                    emit(1, 0, st[name])
                elif name == "p5":
                    emit(1, 1, st["u3"] + st[name])
                    st["u4"] = st["u2"] + st[name]
                elif name == "u5":
                    emit(0, 1, st[name])
            plan = [("p1", 0, None), ("u1", 1, "p1"), ("u2", 5, "p1"), ("u3", 6, "u2"), ("u6", 3, "u3"),
                    ("p5", 4, None), ("u5", 2, "u4")]
            if p5_first:
                plan[4:6] = plan[5], plan[4]
            return [functools.partial(step, *p, d0) for p in plan for d0 in range(0, HALF, ds)]

        def weigh_values(slot, c, early, narrow=False):
            k0, k1, kh = c * L, (c + 1) * L, S - (0 if early is None else NH)
            parts = []
            if k0 < kh:
                parts.append(jnp.exp2(s_v[slot, k0:min(k1, kh), :]))
            if k1 > kh:
                parts.append(early[max(k0, kh) - kh:k1 - kh, :])
            p = _cat(parts)
            return _dot(v_v[c], p.astype(BF16) if early is None or narrow else p)

        def attend(i, nv, early, extra=()):
            nm = S - nv - (0 if early is None else NH)
            keys = key_operand if extra else functools.cache(key_operand)
            for j in range(4):
                q = _cat([q_v[i, j * Dh:(j + 1) * Dh, 0:TQ], jnp.zeros((32 - Dh, TQ), F32)]).astype(BF16)
                steps, queries = [], functools.cache(functools.partial(query_operand, i, j))
                for k0 in range(nm, nm + nv, 2 * KB):
                    def store(r, cols, s, k0=k0):
                        s_v[j % 2, k0 + r:k0 + r + 8, cols] = s
                    steps += score_steps(keys, queries, (k0 - (S - NB)) // KB, store, not extra)
                fill = filler(nm + 24 * NC, steps, extra[j * len(extra) // 4:(j + 1) * len(extra) // 4])
                acc = None
                for c in range(NC):
                    lo, hi = 16 * (c * (nm // 16) // NC), 16 * ((c + 1) * (nm // 16) // NC)
                    s = _dot(_bf16(k_v[lo // 2:hi // 2, :]), q)
                    s_v[j % 2, lo:hi, :] = s
                    fill.tick(s, hi - lo)
                    o = weigh_values(1 - j % 2, c, None if early is None else early(j))
                    acc = o if acc is None else acc + o
                    fill.tick(o, 24)
                o_v[(4 * i + j + 2 * H - 1) % (2 * H)] = acc

        def attend_with_max(t, n):
            hh, cols = n // 4, _multiple(n % 4, L)
            q = q_v[t * NG + hh // 4, 0:Dh, cols]
            for j in range(1, 4):
                q = jnp.where(hh % 4 == j, q_v[t * NG + hh // 4, j * Dh:(j + 1) * Dh, cols], q)
            s = _dot(_bf16(k_v[...]), _cat([q, jnp.zeros((32 - Dh, L), F32)]).astype(BF16))
            p = jnp.exp2(s - jnp.max(s, axis=0, keepdims=True))
            o_v[t % 2 * H + hh, :, cols] = _dot(_cat([v_v[c] for c in range(NC)], 1), p)

        def first_phase(w_v, raw_v, wm_v, h_v, kx_v, wkv_v, wqt_v, wt_v, osem, xsems, wsems):
            cp_wo = pltpu.make_async_copy(wo_hbm, w_v.at[1], osem)

            def x_copy(t):
                return pltpu.make_async_copy(x_hbm.at[:, _multiple(t, TQ)], x_v.at[t], xsems.at[t])

            def unit_copies(u):
                cols = pl.ds(pl.multiple_of(2 * D + u * 2 * L, L), 2 * L)
                return [pltpu.make_async_copy(w.at[:, _multiple(u, 4 * L)], raw_v.at[u % 3, n], wsems.at[u % 3, n])
                        for n, w in enumerate((wg_hbm, wu_hbm, wd_hbm))] + [
                    pltpu.make_async_copy(wm_hbm.at[:, cols], wm_v.at[:, cols], wsems.at[u % 3, 3])]

            def modulation(at, n):
                m = _dot(wkv_v[48:64, :], wm_v[:, pl.ds(at, n)])[0:1]
                col = at + lax.broadcasted_iota(jnp.int32, (1, n), 1)
                within = lambda i: jnp.logical_and(col >= i * D, col < (i + 1) * D)
                m = jnp.where(jnp.logical_or(within(1), within(4)), m + 1.0, m)
                m = m * jnp.where(jnp.logical_or(within(3), within(4)), 0.5, jnp.where(within(5), 2.0, 1.0))
                mod_v[pl.ds(at, n), :] = jnp.broadcast_to(m, (L, n)).T

            def transposed(blk, pin):
                blk = _words(blk)
                head = _cat([pin(blk[0:8, 0:L]), blk[0:8, L:]], 1) if blk.shape[1] > L else pin(blk[0:8])
                return _words(_bf16(_cat([head, blk[8:]])).T)

            def square_steps(w_ref, dst):
                high = lax.broadcasted_iota(jnp.int32, (1, L), 1) >= 64
                minus = lambda a, b: _words(_bf16(a).astype(F32) - _bf16(jnp.where(high, b, 0)).astype(F32))

                def step(n, lo, hi, pin):
                    wt = transposed(_cat([w_ref[lo:lo + 64, :], w_ref[hi:hi + 64, :]]), pin)
                    top, bot = wt[0:D // 4], wt[D // 4:D // 2]
                    if n < 3:
                        dst[:, n * L:(n + 1) * L], dst[:, (n + 4) * L:(n + 5) * L] = top, bot
                    else:
                        dst[:, n * L:(n + 1) * L] = (
                            minus(top, bot) if n == 3 else minus(bot, top) if n == 7 else jnp.where(high, top, bot))
                tiles = [(n, n * L, n * L + 64) for n in range(4)] + [(7, 3 * L, 4 * L), (8, 4 * L - 64, 4 * L)]
                return [functools.partial(step, *t) for t in tiles]

            def key_steps(row, c, d, first=0):
                cols = {}

                def spread(e, pin):
                    rows = jnp.broadcast_to(row(d + e * HALF), (L, L))
                    cols[e] = _words(_cat([pin(rows[0:8]), rows[8:]]).astype(BF16).T)

                def combine(r, pin):
                    a1, a2 = [_bf16(pin(cols[e][8 * r:8 * r + 8])).astype(F32) for e in range(2)]
                    a11, a21, a12, a22 = a1[0:8], a1[8:16], a2[0:8], a2[8:16]
                    s1 = a21 + a22
                    s2 = s1 - a11
                    for p, a in enumerate((a11, a12, a12 - s2, -a22, s1, s2, a11 - a21)):
                        kb_v[8 * c + r, HALF * p + d] = a
                return ([functools.partial(spread, e) for e in range(2)],
                        [functools.partial(combine, r) for r in range(first, 8)])

            def project(t):
                @pl.when(t + 1 < NQ)
                def _():
                    x_copy(jnp.minimum(t + 1, NQ - 1)).wait()

                for at, copies in enumerate(([x_copy(2), x_copy(3)], [cp_wo] + unit_copies(0), unit_copies(1))):
                    @pl.when(t == at)
                    def _():
                        for cp in copies:
                            cp.start()

                @pl.when(t == NQ - 1)
                def _():
                    cp_wo.wait()

                h = h_v[t % 2]
                kv = _dot(wkv_v[0:48, :], h)
                k, v = kv[0:24] * scale, kv[24:48]
                for d in range(Dh):
                    kx_v[d, 0:1, :] = k[d:d + 1, TQ - 2 * L:TQ - L]
                keys = [key_steps(lambda d: k[d:d + 1, TQ - L:], t + 1, d) for d in range(HALF)]
                steps = [lambda pin: None] * 8 + keys[0][0]
                for d in range(HALF):
                    steps += (keys[d + 1][0] if d + 1 < HALF else []) + keys[d][1]

                def emit(r, norm):
                    h_v[(t + 1) % 2, r:r + 16, :] = (norm(r) * mod(1, r, 16, 4) + mod(0, r, 16, 4)).astype(BF16)
                nxt = jnp.minimum(t + 1, NQ - 1)
                fill = filler(9 * D // 2 - 100, steps, _norm_steps(
                    lambda r, n: x_v[nxt, r:r + n, :].astype(F32), D, emit, range(0, D, 16)),
                    square_steps(w_v.at[t // (NQ - 1)], wot_v))
                q2 = norm_v[0, 0:1, 0:L]
                low = {}
                for l, half, q in square_dot(wqt_v, h, (0, 2, 1, 3), fill):
                    up = _cat([q[HALF:], q[:HALF]])
                    parts = {l: q}
                    if l < 2:
                        low[half] = q, up
                    else:
                        t1 = q - low[half][0]
                        parts.update({l + 2: up - t1 - low[half][1], l + 4: t1, l + 6: up - t1, l + 8: up - q})
                    for m, y in parts.items():
                        q_v[pl.ds(t * NG + half * NG // 2, NG // 2), :, m * L:(m + 1) * L] = y.reshape(NG // 2, -1, L)
                    qq = q * q
                    for r in range(0, D // 2, Dh):
                        q2 = jnp.maximum(q2, jnp.sum(qq[r:r + Dh], axis=0, keepdims=True))
                norm_v[0, 0:1, 0:L] = q2
                norm_v[1, 0:1, :] = jnp.maximum(norm_v[1, 0:1, :], jnp.sum(k * k, axis=0, keepdims=True))
                norm_v[2, 0:1, :] = jnp.maximum(norm_v[2, 0:1, :], jnp.max(jnp.abs(v), axis=0, keepdims=True))
                kn = _words(_cat([k, jnp.zeros((L - 24, TQ), F32)]).astype(BF16).T)[:, 0:32]
                vn = jnp.where(lax.broadcasted_iota(jnp.int32, (24, TQ), 0) == Dh, 1.0, v)
                for c in range(4):
                    at = 3 * t + c if c < 3 else 3 * NQ + t
                    k_v[_multiple(at, L // 2), :] = kn[c * L // 2:(c + 1) * L // 2]
                    v_v[at] = vn[:, c * L:(c + 1) * L]

            def weight_steps(u):
                slot = u % 3
                lane = lax.broadcasted_iota(jnp.int32, (8, L), 1)

                def transpose(w, half, kind, pin):
                    rows = lambda r, m, n: raw_v[slot, w, pl.ds(half * D // 2 + r, m), n * L:(n + 1) * L]
                    if kind < 4:
                        blk = rows(0, L, kind)
                    elif kind < 8:
                        blk = _cat([rows(L if m == kind - 4 else 160 + 32 * m, 32, kind - 4) for m in range(4)])
                    else:
                        blk = _cat([rows(160 + 32 * m, 32, m) for m in range(4)])
                    wt_v[w, half, kind] = transposed(blk, pin)

                def combine(kind, r, pin):
                    block = lambda row, half, k: wt_v[r // 8 % 2, half, k, pl.ds(r // 16 * 16 + 8 * row, 8), :]

                    def operand(row, half):
                        x = _bf16(pin(block(row, half, kind))).astype(F32)
                        if 4 <= kind < 8:
                            x -= _bf16(jnp.where(lane // 32 == kind - 4, 0, block(row, half, 8))).astype(F32)
                        return x
                    rows = pl.ds(pl.multiple_of(u * (L // 2) + r, 8), 8)
                    y = _strassen_lhs([[operand(row, half) for half in range(2)] for row in range(2)])
                    if 4 <= kind < 8:
                        y = _all_words(y)
                    else:
                        y = _all_words(y[0:2] + y[4:7])
                        y[2:2] = [block(e, e, kind) for e in range(2)]
                    for i in range(7):
                        if kind == 8:
                            ws_v[i, rows, :] = y[i]
                        else:
                            wa_v[i, kind % 4, rows, kind // 4 * L:(kind // 4 + 1) * L] = y[i]

                outer = {}

                def down_outer(r, a, b, pin):
                    def operand(q, n):
                        x = raw_v[slot, 2, pl.ds(q * D // 4 + 2 * r, 16), n * L:(n + 1) * L]
                        return _bf16(pin(_words(x))).astype(F32)
                    outer[a, b] = _strassen_lhs([[operand(a + 2 * q, 2 * b + n) for n in range(2)] for q in range(2)])

                def down_inner(r, i, pin):
                    y = _words(_cat(_strassen_lhs([[pin(outer[a, b][i]) if a == b else outer[a, b][i]
                                                    for b in range(2)] for a in range(2)]), 1))
                    for k in range(7):
                        wd_v[7 * i + k, u, r:r + 8, :] = y[:, k * L:(k + 1) * L]

                steps = []
                kinds = [8, 0, 4, 1, 5, 2, 6, 3, 7]
                for n in range(10):
                    for e in range(8):
                        if n < 9 and e % 2 == 0:
                            steps.append(functools.partial(transpose, e // 4, e // 2 % 2, kinds[n]))
                        if n > 0:
                            steps.append(functools.partial(combine, kinds[n - 1], 8 * e))
                late = []
                for r in range(0, D // 8, 8):
                    late += [functools.partial(down_outer, r, a, b) for a in range(2) for b in range(2)]
                    late += [functools.partial(down_inner, r, i) for i in range(7)]
                mods = [lambda pin, n=n: modulation(pl.multiple_of(2 * D + (2 * u + n) * L, L), L) for n in range(2)]
                keys = key_steps(lambda d: kx_v[d, 0:1, :], 0, u, (NB - NV1 - NH) // KB)
                steps = steps[:20] + mods[:1] + steps[20:]
                late = keys[0] + late[:30] + keys[1] + late[30:60] + mods[1:] + late[60:]
                return steps + late + [lambda pin: None] * 4

            def prologue(wk_v, wv_v, c_v, sems):
                cp_c, cp_wq, cp_wk, cp_wv, cp_wm = [
                    pltpu.make_async_copy(src, dst, sems.at[n]) for n, (src, dst) in enumerate((
                        (c_hbm, c_v), (wq_hbm, w_v.at[0]), (wk_hbm, wk_v), (wv_hbm, wv_v),
                        (wm_hbm.at[:, pl.ds(0, 2 * D)], wm_v.at[:, pl.ds(0, 2 * D)])))]
                for cp in (cp_c, x_copy(0), cp_wm):
                    cp.start()
                zero_v[...] = jnp.zeros_like(zero_v)
                norm_v[...] = jnp.zeros_like(norm_v)
                s_v[1] = jnp.zeros(s_v.shape[1:], F32)
                x_copy(0).wait()
                for cp in (cp_wq, cp_wk, cp_wv):
                    cp.start()

                def keep(r, norm):
                    x1_v[r:r + 16, :] = norm(r)
                _run(_norm_steps(lambda r, n: x_v[0, r:r + n, :].astype(F32), D, keep, range(0, D, 16)))
                x_copy(1).start()
                cp_c.wait()
                cp_wm.wait()
                c = c_v[...].astype(F32)
                wkv_v[48:64, :] = jnp.broadcast_to(c * jax.nn.sigmoid(c), (16, D)).astype(BF16)
                modulation(0, 2 * D)
                h_v[0] = (x1_v[...] * mod(1, 0, D, 4) + mod(0, 0, D, 4)).astype(BF16)
                for cp in (cp_wq, cp_wk, cp_wv):
                    cp.wait()
                _run(square_steps(w_v.at[0], wqt_v))
                pad = jnp.zeros((24 - Dh, D), F32)
                wkv_v[0:48, :] = _cat([wk_v[...].astype(F32), pad, wv_v[...].astype(F32), pad]).astype(BF16)

            pl.run_scoped(prologue, pltpu.VMEM((Dh, D), BF16), pltpu.VMEM((Dh, D), BF16),
                          pltpu.VMEM((1, D), BF16), pltpu.SemaphoreType.DMA((5,)))
            _loop(NQ, project)

            def first_tile(u):
                for cp in unit_copies(u):
                    cp.wait()

                @pl.when(u + 2 < NU)
                def _():
                    for cp in unit_copies(jnp.minimum(u + 2, NU - 1)):
                        cp.start()
                attend(u, NV0, None, weight_steps(u))
            _loop(NU, first_tile)

        pl.run_scoped(
            first_phase,
            pltpu.VMEM((2, D, D), BF16), pltpu.VMEM((3, 3, D, 4 * L), BF16),
            pltpu.VMEM((D, 6 * D), BF16), pltpu.VMEM((2, D, TQ), BF16), pltpu.VMEM((Dh, 8, L), F32),
            pltpu.VMEM((64, D), BF16), pltpu.VMEM((D // 4, 9 * L), U32), pltpu.VMEM((2, 2, 9, L // 2, L), U32),
            pltpu.SemaphoreType.DMA(()), pltpu.SemaphoreType.DMA((NQ,)), pltpu.SemaphoreType.DMA((3, 4)))

        bound = jnp.max(norm_v[0, 0:1, :], axis=1, keepdims=True) * norm_v[1, 0:1, :]
        ok = jnp.logical_and(bound <= SAFE_SCORE ** 2, norm_v[2, 0:1, :] <= SAFE_VALUE)
        safe = jnp.max(jnp.where(ok, 0.0, 1.0)) < 0.5

        def second_phase(p_v, hb_v, act_v, out_v, sems):
            def out_copy(t, half):
                rows = pl.ds(half * D // 2, D // 2)
                return pltpu.make_async_copy(out_v.at[t, rows], out_hbm.at[rows, _multiple(t, TQ)], sems.at[t, half])

            def early_scores(t, reuse, first_head, heads, first_key, keys, cycles):
                steps, operands = [], reuse(key_operand)
                for e in range(heads):
                    hh = first_head + e
                    queries = reuse(functools.partial(
                        query_operand, jnp.minimum((t + 1) * NG + (hh + 3) // 4, NQ * NG - 1), (e + 3) % 4))
                    for k0 in range(first_key, first_key + keys, 2 * KB):
                        def store(r, cols, s, k0=k0, hh=hh):
                            p_v[hh, k0 + r:k0 + r + 8, cols] = jnp.exp2(s)
                        steps += score_steps(operands, queries, (NB - NH + k0) // KB, store)
                return filler(cycles, steps)

            def project_heads(t):
                heads = o_v.at[pl.ds(t % 2 * H, H)]
                inv = [1.0 / heads[g:g + 8, Dh, :] for g in range(0, H, 8)]
                steps = []
                for pair in range(2):
                    cols = slice(2 * pair * L, 2 * (pair + 1) * L)
                    o = _cat([heads[hh, 0:Dh, cols] * inv[hh // 8][hh % 8:hh % 8 + 1, cols] for hh in range(H)])
                    for l, half, a in square_dot(wot_v, o.astype(BF16), (0, 1), filler(9 * D // 4, steps)):
                        r, c = half * D // 2, slice((2 * pair + l) * L, (2 * pair + l + 1) * L)
                        x1_v[r:r + D // 2, c] = x_v[t, r:r + D // 2, c].astype(F32) + mod(2, r, D // 2, 1) * a

                    def emit(r, norm, pair=pair):
                        h = [norm(r0) * mod(4, r0, 16, 2) + mod(3, r0, 16, 2) for r0 in (r, r + D // 2)]
                        y = _words(_cat(_strassen_rhs([[hk[:, 0:L], hk[:, L:]] for hk in h]), 1))
                        for i in range(7):
                            hb_v[i, r // 2:r // 2 + 8, pair * L:(pair + 1) * L] = y[:, i * L:(i + 1) * L]
                    steps = _norm_steps(lambda r, n, cols=cols: x1_v[r:r + n, cols], D, emit, range(0, D // 2, 16))
                _run(steps)

            def gate_up(t, it):
                room = ((96, 80, 96, 96, 80, 80, 80), (96, 60, 96, 96, 60, 60, 60))
                fill = early_scores(t, functools.cache, it * (H // GI), H // GI, 0, NH_UP,
                                    UG * (7 * 24 + 2 * sum(room[0] + room[1])))
                for block in range(UG):
                    rows = _multiple(it * UG + block, RB // 2)
                    shared = [[None] * 2 for _ in range(2)]
                    for i in range(7):
                        m = _dot(_bf16(ws_v[i, rows, :]), _bf16(hb_v[i, 80:144, :]))
                        fill.tick(m, 24)
                        _strassen_add(shared, i, m)
                    acts = []
                    for n in range(4):
                        c = [list(r) for r in shared]
                        for at, i in enumerate((2, 4, 0, 1, 5, 3, 6)):
                            rhs = [hb_v[i, 0:64, :]] + [
                                hb_v[i, pl.ds(64 if m == n else 80 + 16 * m, 16), :] for m in range(4)]
                            m = _dot(_bf16(wa_v[i, n, rows, :]), _bf16(_cat(rhs)))
                            fill.tick(m, room[n % 2][at])
                            _strassen_add(c, i, m)
                        acts.append([_cat([_swiglu(c[row][k][r:r + 16], c[row][k][r + 16:r + 32])
                                          for r in range(0, RB, 32) for row in range(2)]) for k in range(2)])
                        if n % 2 == 1:
                            for i, y in enumerate(_strassen_rhs(acts[n - 1:])):
                                act_v[i, n // 2, _multiple(it * UG + block, RB), :] = y

            def down(t):
                fill = early_scores(t, lambda f: f, 0, H, NH_UP, NH_DOWN, 49 * NU * D // 16)
                y = [[[[None] * 2 for _ in range(2)] for _ in range(2)] for _ in range(2)]
                for i in (2, 3, 4, 1, 0, 6, 5):
                    c = [[None] * 2 for _ in range(2)]
                    for k in range(7):
                        acc = None
                        for u0, u1 in ((0, 4), (4, 5), (5, NU)):
                            b = _strassen_rhs([[act_v[i, r, u0 * L:u1 * L, n * L:(n + 1) * L] for n in range(2)]
                                               for r in range(2)])[k]
                            m = _dot(_bf16(_cat([wd_v[7 * i + k, u] for u in range(u0, u1)], 1)), b.astype(BF16))
                            fill.tick(m, (u1 - u0) * D // 16)
                            acc = m if acc is None else acc + m
                        _strassen_add(c, k, acc)
                    for r in range(2):
                        for n in range(2):
                            _strassen_add(y[r][n], i, c[r][n])
                    if i in (6, 5):
                        half = 6 - i
                        rows = slice(half * D // 2, (half + 1) * D // 2)
                        ffn = _cat([_cat([y[r][n // 2][half][n % 2] for n in range(4)], 1) for r in range(2)])
                        out_v[t, rows, :] = (x1_v[rows, :] + mod(5, rows.start, D // 2, 4) * ffn).astype(BF16)
                        out_copy(t, half).start()

            def tile(t):
                @pl.when(safe)
                def _():
                    _loop(jnp.where(t == 0, 0, jnp.where(t == NQ - 1, NG - 1, NG)),
                          lambda g: attend(t * NG + 1 + g, NV1, lambda j: p_v.at[4 * g + j]))

                    def last_head(_):
                        o_v[2 * H - 1] = sum(weigh_values(1, c, p_v.at[H - 4], True) for c in range(NC))
                    _loop(jnp.where(t == NQ - 1, 1, 0), last_head)

                @pl.when(jnp.logical_not(safe))
                def _():
                    _loop(4 * H, lambda n: attend_with_max(t, n))

                project_heads(t)
                _loop(GI, lambda it: gate_up(t, it))
                down(t)

            _loop(NQ, tile)
            for t in range(NQ):
                for half in range(2):
                    out_copy(t, half).wait()

        pl.run_scoped(
            second_phase,
            pltpu.VMEM((H, NH, TQ), F32), pltpu.VMEM((7, D // 4, 2 * L), U32),
            pltpu.VMEM((7, 2, NU * L, 2 * L), F32), pltpu.VMEM((NQ, D, TQ), BF16),
            pltpu.SemaphoreType.DMA((NQ, 2)))

    scratch = [
        pltpu.VMEM((NQ, D, TQ), BF16),
        pltpu.VMEM((D, TQ), F32),
        pltpu.VMEM((6 * D, L), F32),
        pltpu.VMEM((3, 8, TQ), F32),
        pltpu.VMEM((16, L), jnp.int32),
        pltpu.VMEM((D // 4, 9 * L), U32),
        pltpu.VMEM((NQ * NG, 4 * Dh, 3 * TQ), F32),
        pltpu.VMEM((S // 2, 32), U32),
        pltpu.VMEM((NB // KB, 66, 8, L), F32),
        pltpu.VMEM((NC, 24, L), F32),
        pltpu.VMEM((2, S, TQ), F32),
        pltpu.VMEM((2 * H, 24, TQ), F32),
        pltpu.VMEM((7, 4, NU * L // 2, 2 * L), U32),
        pltpu.VMEM((7, NU * L // 2, L), U32),
        pltpu.VMEM((51, NU, D // 8, L), U32),
    ]
    return kernel, scratch


@jax.jit
def pallas_adaLN_cond__grouped_kv_mqa__swiglu_ffn__prompt_kernel(
    A_x: jax.Array,
    A_wq: jax.Array,
    A_wk: jax.Array,
    A_wv: jax.Array,
    A_wo: jax.Array,
    B_x: jax.Array,
    B_w_gate: jax.Array,
    B_w_up: jax.Array,
    B_w_down: jax.Array,
    c: jax.Array,
    w_mod: jax.Array,
):
    del B_x
    _, S, D = A_x.shape
    kernel, scratch = _make_kernel(S, D, B_w_gate.shape[1])
    out_t = pl.pallas_call(
        kernel,
        in_specs=[pl.BlockSpec(memory_space=pl.ANY)] * 10,
        out_specs=pl.BlockSpec(memory_space=pl.ANY),
        out_shape=jax.ShapeDtypeStruct((D, S), A_x.dtype),
        scratch_shapes=scratch,
        compiler_params=pltpu.CompilerParams(vmem_limit_bytes=122 * 2 ** 20),
        name="adaln_block",
    )(A_x.reshape(S, D).T, A_wq, A_wk.T, A_wv.T, A_wo, B_w_gate, B_w_up, B_w_down.T, c, w_mod)
    return out_t.T.reshape(1, S, D)
```

```python
import functools
import math

import jax
import jax.numpy as jnp
from jax import lax
import jax.experimental.pallas as pl
import jax.experimental.pallas.tpu as pltpu

BF16, F32, U32 = jnp.bfloat16, jnp.float32, jnp.uint32
H = 32
EPS = 1e-5
L = 128
TQ = 4 * L
KB = 16
SAFE_SCORE = 60.0
SAFE_VALUE = 2.0 ** 50


def _dot(a, b):
    return jnp.dot(a, b, preferred_element_type=F32)


def _cat(xs, axis=0):
    return xs[0] if len(xs) == 1 else jnp.concatenate(xs, axis=axis)


def _words(x):
    return pltpu.bitcast(x.astype(BF16), U32)


def _all_words(xs):
    y = _words(_cat(xs, 1))
    return [y[:, n * L:(n + 1) * L] for n in range(len(xs))]


def _bf16(x):
    return pltpu.bitcast(x, BF16)


def _multiple(i, n):
    return pl.ds(pl.multiple_of(i * n, n), n)


def _strassen_lhs(a):
    (a11, a12), (a21, a22) = a
    return [a11 + a22, a21 + a22, a11, a22, a11 + a12, a21 - a11, a12 - a22]


def _strassen_rhs(b):
    (b11, b12), (b21, b22) = b
    return [b11 + b22, b11, b12 - b22, b21 - b11, b22, b11 + b12, b21 + b22]


def _strassen_add(c, i, m):
    for r, k, sign in (((0, 0, 1), (1, 1, 1)), ((1, 0, 1), (1, 1, -1)), ((0, 1, 1), (1, 1, 1)),
                       ((0, 0, 1), (1, 0, 1)), ((0, 0, -1), (0, 1, 1)), ((1, 1, 1),), ((0, 0, 1),))[i]:
        if c[r][k] is None:
            assert sign > 0
            c[r][k] = m
        else:
            c[r][k] = c[r][k] + m if sign > 0 else c[r][k] - m


def _swiglu(g, u):
    return (g + g * jnp.tanh(g)) * u


def _norm_steps(load, n, emit, rows):
    st = {}

    def fold(key, x):
        x = jnp.sum(x.reshape(-1, 8, x.shape[1]), axis=0)
        st[key] = st[key] + x if key in st else x

    def mean(key):
        return jnp.sum(st[key], axis=0, keepdims=True) * (1.0 / n)

    def sums(r, pin):
        fold("sum", load(r, 64))
        if r + 64 == n:
            st["mean"] = jnp.broadcast_to(mean("sum"), st["sum"].shape)

    def squares(r, pin):
        d = load(r, 64) - _cat([pin(st["mean"])] * 8)
        fold("sq", d * d)
        if r + 64 == n:
            st["rstd"] = lax.rsqrt(mean("sq") + EPS)

    def write(r, pin):
        mu = _cat([pin(st["mean"])] * 2)
        emit(r, lambda r0: (load(r0, 16) - mu) * st["rstd"])

    return ([functools.partial(sums, r) for r in range(0, n, 64)]
            + [functools.partial(squares, r) for r in range(0, n, 64)]
            + [functools.partial(write, r) for r in rows])


def _run(steps):
    for step in steps:
        step(lambda x: x)


def _tile(x, shape):
    return _cat([_cat([x] * (shape[1] // L), 1)] * (shape[0] // 8))


class _Filler:
    def __init__(self, never, cycles, *streams):
        self.never = functools.cache(functools.partial(_tile, never))
        self.now = 0
        due = [(e * cycles // len(st), n, e, step) for n, st in enumerate(streams) for e, step in enumerate(st)]
        self.due = sorted(due, key=lambda d: d[:3], reverse=True)

    def tick(self, result, cycles):
        while self.due and self.due[-1][0] < self.now + cycles:
            at, _, _, step = self.due.pop()
            r = 8 * ((at - self.now) * (result.shape[0] // 8) // cycles)
            step(functools.partial(self.pin, result[r:r + 8, 0:L]))
        self.now += cycles

    def pin(self, mark, x):
        if x.dtype != mark.dtype:
            mark = pltpu.bitcast(mark, x.dtype)
        return lax.select(self.never(x.shape), _tile(mark, x.shape), x)


def _loop(n, f):
    def body(i, carry):
        f(i)
        return carry
    lax.fori_loop(0, n, body, 0)


def _make_kernel(S, D, F):
    assert (S, D, F) == (2048, 576, 4608)
    Dh = D // H
    HALF = Dh // 2
    NQ = S // TQ
    NG = H // 4
    NC = S // L
    NU = F // (4 * L)
    RB, UG = 96, 6
    GI = NU * L // (RB * UG)
    NV0, NV1, NH_UP, NH_DOWN = 224, 352, 160, 64
    NH = NH_UP + NH_DOWN
    NB = (NQ + 1) * L
    scale = float(Dh ** -0.5 * math.log2(math.e))

    def kernel(x_hbm, wq_hbm, wk_hbm, wv_hbm, wo_hbm, wg_hbm, wu_hbm, wd_hbm, c_hbm, wm_hbm, out_hbm,
               x_v, x1_v, mod_v, norm_v, zero_v, wot_v, q_v, k_v, kb_v, v_v, s_v, o_v, wa_v, ws_v, wd_v):

        def filler(cycles, *streams):
            return _Filler(zero_v[0:8, :] != 0, cycles, *streams)

        def mod(i, r, n, tiles):
            return _cat([mod_v[i * D + r:i * D + r + n, :]] * tiles, 1)

        def square_dot(w_ref, a, order, fill):
            shared = _dot(_bf16(w_ref[:, 8 * L:9 * L]), a[4 * L - 64:D])
            fill.tick(shared, len(order) * D // 8)
            for l in order:
                cols = slice(l * L, (l + 1) * L)
                for half, rhs in enumerate((a[0:4 * L], _cat([a[0:4 * L - 64], a[4 * L:D]]))):
                    y = _dot(_bf16(w_ref[:, 4 * half * L:4 * (half + 1) * L]), rhs[:, cols])
                    fill.tick(y, D // 2)
                    yield l, half, y + shared[:, cols]

        def key_operand(b, e):
            k = kb_v[b // 2, e]
            return _cat([k, k], 1)

        def query_operand(i, j, r, l):
            r += j * Dh
            q = _cat([jnp.broadcast_to(q_v[i, r:r + 1, m * L:(m + 1) * L], (8, L)) for m in (l, l + 1)], 1)
            return q, _cat([q, q])

        def score_steps(keys, queries, b, store, p5_first=False):
            st = {}
            q_at = [(0, 0), (HALF, 0), (HALF, 2), (0, 4), (0, 6), (0, 8), (0, 10)]
            ds = 5

            def emit(row, col, s):
                for m in range(2):
                    store(KB * m + 8 * row, slice(2 * col * L, 2 * (col + 1) * L), s[8 * m:8 * m + 8])

            def step(name, p, start, d0, pin):
                for d in range(d0, min(d0 + ds, HALF)):
                    k = keys(b, HALF * p + d)
                    q, qq = queries(q_at[p][0] + d, q_at[p][1])
                    t = k * (_cat([pin(q)] * 2) if d == d0 else qq)
                    prev = name if d else start
                    st[name] = t if prev is None else st[prev] + t
                if d0 + ds < HALF:
                    return
                if name == "u1":
                    emit(0, 0, st[name])
                elif name == "u6":
                    emit(1, 0, st[name])
                elif name == "p5":
                    emit(1, 1, st["u3"] + st[name])
                    st["u4"] = st["u2"] + st[name]
                elif name == "u5":
                    emit(0, 1, st[name])
            plan = [("p1", 0, None), ("u1", 1, "p1"), ("u2", 5, "p1"), ("u3", 6, "u2"), ("u6", 3, "u3"),
                    ("p5", 4, None), ("u5", 2, "u4")]
            if p5_first:
                plan[4:6] = plan[5], plan[4]
            return [functools.partial(step, *p, d0) for p in plan for d0 in range(0, HALF, ds)]

        def weigh_values(slot, c, early, narrow=False):
            k0, k1, kh = c * L, (c + 1) * L, S - (0 if early is None else NH)
            parts = []
            if k0 < kh:
                parts.append(jnp.exp2(s_v[slot, k0:min(k1, kh), :]))
            if k1 > kh:
                parts.append(early[max(k0, kh) - kh:k1 - kh, :])
            p = _cat(parts)
            return _dot(v_v[c], p.astype(BF16) if early is None or narrow else p)

        def attend(i, nv, early, extra=()):
            nm = S - nv - (0 if early is None else NH)
            keys = key_operand if extra else functools.cache(key_operand)
            for j in range(4):
                q = _cat([q_v[i, j * Dh:(j + 1) * Dh, 0:TQ], jnp.zeros((32 - Dh, TQ), F32)]).astype(BF16)
                steps, queries = [], functools.cache(functools.partial(query_operand, i, j))
                for k0 in range(nm, nm + nv, 2 * KB):
                    def store(r, cols, s, k0=k0):
                        s_v[j % 2, k0 + r:k0 + r + 8, cols] = s
                    steps += score_steps(keys, queries, (k0 - (S - NB)) // KB, store, not extra)
                fill = filler(nm + 24 * NC, steps, extra[j * len(extra) // 4:(j + 1) * len(extra) // 4])
                acc = None
                for c in range(NC):
                    lo, hi = 16 * (c * (nm // 16) // NC), 16 * ((c + 1) * (nm // 16) // NC)
                    s = _dot(_bf16(k_v[lo // 2:hi // 2, :]), q)
                    s_v[j % 2, lo:hi, :] = s
                    fill.tick(s, hi - lo)
                    o = weigh_values(1 - j % 2, c, None if early is None else early(j))
                    acc = o if acc is None else acc + o
                    fill.tick(o, 24)
                o_v[(4 * i + j + 2 * H - 1) % (2 * H)] = acc

        def attend_with_max(t, n):
            hh, cols = n // 4, _multiple(n % 4, L)
            q = q_v[t * NG + hh // 4, 0:Dh, cols]
            for j in range(1, 4):
                q = jnp.where(hh % 4 == j, q_v[t * NG + hh // 4, j * Dh:(j + 1) * Dh, cols], q)
            s = _dot(_bf16(k_v[...]), _cat([q, jnp.zeros((32 - Dh, L), F32)]).astype(BF16))
            p = jnp.exp2(s - jnp.max(s, axis=0, keepdims=True))
            o_v[t % 2 * H + hh, :, cols] = _dot(_cat([v_v[c] for c in range(NC)], 1), p)

        def first_phase(w_v, raw_v, wm_v, h_v, kx_v, wkv_v, wqt_v, wt_v, osem, xsems, wsems):
            cp_wo = pltpu.make_async_copy(wo_hbm, w_v.at[1], osem)

            def x_copy(t):
                return pltpu.make_async_copy(x_hbm.at[:, _multiple(t, TQ)], x_v.at[t], xsems.at[t])

            def unit_copies(u):
                cols = pl.ds(pl.multiple_of(2 * D + u * 2 * L, L), 2 * L)
                return [pltpu.make_async_copy(w.at[:, _multiple(u, 4 * L)], raw_v.at[u % 3, n], wsems.at[u % 3, n])
                        for n, w in enumerate((wg_hbm, wu_hbm, wd_hbm))] + [
                    pltpu.make_async_copy(wm_hbm.at[:, cols], wm_v.at[:, cols], wsems.at[u % 3, 3])]

            def modulation(at, n):
                m = _dot(wkv_v[48:64, :], wm_v[:, pl.ds(at, n)])[0:1]
                col = at + lax.broadcasted_iota(jnp.int32, (1, n), 1)
                within = lambda i: jnp.logical_and(col >= i * D, col < (i + 1) * D)
                m = jnp.where(jnp.logical_or(within(1), within(4)), m + 1.0, m)
                m = m * jnp.where(jnp.logical_or(within(3), within(4)), 0.5, jnp.where(within(5), 2.0, 1.0))
                mod_v[pl.ds(at, n), :] = jnp.broadcast_to(m, (L, n)).T

            def transposed(blk, pin):
                blk = _words(blk)
                head = _cat([pin(blk[0:8, 0:L]), blk[0:8, L:]], 1) if blk.shape[1] > L else pin(blk[0:8])
                return _words(_bf16(_cat([head, blk[8:]])).T)

            def square_steps(w_ref, dst):
                high = lax.broadcasted_iota(jnp.int32, (1, L), 1) >= 64
                minus = lambda a, b: _words(_bf16(a).astype(F32) - _bf16(jnp.where(high, b, 0)).astype(F32))

                def step(n, lo, hi, pin):
                    wt = transposed(_cat([w_ref[lo:lo + 64, :], w_ref[hi:hi + 64, :]]), pin)
                    top, bot = wt[0:D // 4], wt[D // 4:D // 2]
                    if n < 3:
                        dst[:, n * L:(n + 1) * L], dst[:, (n + 4) * L:(n + 5) * L] = top, bot
                    else:
                        dst[:, n * L:(n + 1) * L] = (
                            minus(top, bot) if n == 3 else minus(bot, top) if n == 7 else jnp.where(high, top, bot))
                tiles = [(n, n * L, n * L + 64) for n in range(4)] + [(7, 3 * L, 4 * L), (8, 4 * L - 64, 4 * L)]
                return [functools.partial(step, *t) for t in tiles]

            def key_steps(row, c, d, first=0):
                cols = {}

                def spread(e, pin):
                    rows = jnp.broadcast_to(row(d + e * HALF), (L, L))
                    cols[e] = _words(_cat([pin(rows[0:8]), rows[8:]]).astype(BF16).T)

                def combine(r, pin):
                    a1, a2 = [_bf16(pin(cols[e][8 * r:8 * r + 8])).astype(F32) for e in range(2)]
                    a11, a21, a12, a22 = a1[0:8], a1[8:16], a2[0:8], a2[8:16]
                    s1 = a21 + a22
                    s2 = s1 - a11
                    for p, a in enumerate((a11, a12, a12 - s2, -a22, s1, s2, a11 - a21)):
                        kb_v[4 * c + r // 2, HALF * p + d, pl.ds(r % 2 * 8, 8), :] = a
                return ([functools.partial(spread, e) for e in range(2)],
                        [functools.partial(combine, r) for r in range(first, 8)])

            def project(t):
                @pl.when(t + 1 < NQ)
                def _():
                    x_copy(jnp.minimum(t + 1, NQ - 1)).wait()

                for at, copies in enumerate(([x_copy(2), x_copy(3)], [cp_wo] + unit_copies(0), unit_copies(1))):
                    @pl.when(t == at)
                    def _():
                        for cp in copies:
                            cp.start()

                @pl.when(t == NQ - 1)
                def _():
                    cp_wo.wait()

                h = h_v[t % 2]
                kv = _dot(wkv_v[0:48, :], h)
                k, v = kv[0:24] * scale, kv[24:48]
                for d in range(Dh):
                    kx_v[d, 0:1, :] = k[d:d + 1, TQ - 2 * L:TQ - L]
                keys = [key_steps(lambda d: k[d:d + 1, TQ - L:], t + 1, d) for d in range(HALF)]
                steps = [lambda pin: None] * 8 + keys[0][0]
                for d in range(HALF):
                    steps += (keys[d + 1][0] if d + 1 < HALF else []) + keys[d][1]

                def emit(r, norm):
                    h_v[(t + 1) % 2, r:r + 16, :] = (norm(r) * mod(1, r, 16, 4) + mod(0, r, 16, 4)).astype(BF16)
                nxt = jnp.minimum(t + 1, NQ - 1)
                fill = filler(9 * D // 2 - 100, steps, _norm_steps(
                    lambda r, n: x_v[nxt, r:r + n, :].astype(F32), D, emit, range(0, D, 16)),
                    square_steps(w_v.at[t // (NQ - 1)], wot_v))
                q2 = norm_v[0, 0:1, 0:L]
                low = {}
                for l, half, q in square_dot(wqt_v, h, (0, 2, 1, 3), fill):
                    up = _cat([q[HALF:], q[:HALF]])
                    parts = {l: q}
                    if l < 2:
                        low[half] = q, up
                    else:
                        t1 = q - low[half][0]
                        parts.update({l + 2: up - t1 - low[half][1], l + 4: t1, l + 6: up - t1, l + 8: up - q})
                    for m, y in parts.items():
                        q_v[pl.ds(t * NG + half * NG // 2, NG // 2), :, m * L:(m + 1) * L] = y.reshape(NG // 2, -1, L)
                    qq = q * q
                    for r in range(0, D // 2, Dh):
                        q2 = jnp.maximum(q2, jnp.sum(qq[r:r + Dh], axis=0, keepdims=True))
                norm_v[0, 0:1, 0:L] = q2
                norm_v[1, 0:1, :] = jnp.maximum(norm_v[1, 0:1, :], jnp.sum(k * k, axis=0, keepdims=True))
                norm_v[2, 0:1, :] = jnp.maximum(norm_v[2, 0:1, :], jnp.max(jnp.abs(v), axis=0, keepdims=True))
                kn = _words(_cat([k, jnp.zeros((L - 24, TQ), F32)]).astype(BF16).T)[:, 0:32]
                vn = jnp.where(lax.broadcasted_iota(jnp.int32, (24, TQ), 0) == Dh, 1.0, v)
                for c in range(4):
                    at = 3 * t + c if c < 3 else 3 * NQ + t
                    k_v[_multiple(at, L // 2), :] = kn[c * L // 2:(c + 1) * L // 2]
                    v_v[at] = vn[:, c * L:(c + 1) * L]

            def weight_steps(u):
                slot = u % 3
                lane = lax.broadcasted_iota(jnp.int32, (8, L), 1)

                def transpose(w, half, kind, pin):
                    rows = lambda r, m, n: raw_v[slot, w, pl.ds(half * D // 2 + r, m), n * L:(n + 1) * L]
                    if kind < 4:
                        blk = rows(0, L, kind)
                    elif kind < 8:
                        blk = _cat([rows(L if m == kind - 4 else 160 + 32 * m, 32, kind - 4) for m in range(4)])
                    else:
                        blk = _cat([rows(160 + 32 * m, 32, m) for m in range(4)])
                    wt_v[w, half, kind] = transposed(blk, pin)

                def combine(kind, r, pin):
                    block = lambda row, half, k: wt_v[r // 8 % 2, half, k, pl.ds(r // 16 * 16 + 8 * row, 8), :]

                    def operand(row, half):
                        x = _bf16(pin(block(row, half, kind))).astype(F32)
                        if 4 <= kind < 8:
                            x -= _bf16(jnp.where(lane // 32 == kind - 4, 0, block(row, half, 8))).astype(F32)
                        return x
                    rows = pl.ds(pl.multiple_of(u * (L // 2) + r, 8), 8)
                    y = _strassen_lhs([[operand(row, half) for half in range(2)] for row in range(2)])
                    if 4 <= kind < 8:
                        y = _all_words(y)
                    else:
                        y = _all_words(y[0:2] + y[4:7])
                        y[2:2] = [block(e, e, kind) for e in range(2)]
                    for i in range(7):
                        if kind == 8:
                            ws_v[i, rows, :] = y[i]
                        else:
                            wa_v[i, kind % 4, rows, kind // 4 * L:(kind // 4 + 1) * L] = y[i]

                outer = {}

                def down_outer(r, a, b, pin):
                    def operand(q, n):
                        x = raw_v[slot, 2, pl.ds(q * D // 4 + 2 * r, 16), n * L:(n + 1) * L]
                        return _bf16(pin(_words(x))).astype(F32)
                    outer[a, b] = _strassen_lhs([[operand(a + 2 * q, 2 * b + n) for n in range(2)] for q in range(2)])

                def down_inner(r, i, pin):
                    y = _words(_cat(_strassen_lhs([[pin(outer[a, b][i]) if a == b else outer[a, b][i]
                                                    for b in range(2)] for a in range(2)]), 1))
                    for k in range(7):
                        wd_v[7 * i + k, u, r:r + 8, :] = y[:, k * L:(k + 1) * L]

                steps = []
                kinds = [8, 0, 4, 1, 5, 2, 6, 3, 7]
                for n in range(10):
                    for e in range(8):
                        if n < 9 and e % 2 == 0:
                            steps.append(functools.partial(transpose, e // 4, e // 2 % 2, kinds[n]))
                        if n > 0:
                            steps.append(functools.partial(combine, kinds[n - 1], 8 * e))
                late = []
                for r in range(0, D // 8, 8):
                    late += [functools.partial(down_outer, r, a, b) for a in range(2) for b in range(2)]
                    late += [functools.partial(down_inner, r, i) for i in range(7)]
                mods = [lambda pin, n=n: modulation(pl.multiple_of(2 * D + (2 * u + n) * L, L), L) for n in range(2)]
                keys = key_steps(lambda d: kx_v[d, 0:1, :], 0, u, (NB - NV1 - NH) // KB)
                steps = steps[:20] + mods[:1] + steps[20:]
                late = keys[0] + late[:30] + keys[1] + late[30:60] + mods[1:] + late[60:]
                return steps + late + [lambda pin: None] * 4

            def prologue(wk_v, wv_v, c_v, sems):
                cp_c, cp_wq, cp_wk, cp_wv, cp_wm = [
                    pltpu.make_async_copy(src, dst, sems.at[n]) for n, (src, dst) in enumerate((
                        (c_hbm, c_v), (wq_hbm, w_v.at[0]), (wk_hbm, wk_v), (wv_hbm, wv_v),
                        (wm_hbm.at[:, pl.ds(0, 2 * D)], wm_v.at[:, pl.ds(0, 2 * D)])))]
                for cp in (cp_c, x_copy(0), cp_wm):
                    cp.start()
                zero_v[...] = jnp.zeros_like(zero_v)
                norm_v[...] = jnp.zeros_like(norm_v)
                s_v[1] = jnp.zeros(s_v.shape[1:], F32)
                x_copy(0).wait()
                for cp in (cp_wq, cp_wk, cp_wv):
                    cp.start()

                def keep(r, norm):
                    x1_v[r:r + 16, :] = norm(r)
                _run(_norm_steps(lambda r, n: x_v[0, r:r + n, :].astype(F32), D, keep, range(0, D, 16)))
                x_copy(1).start()
                cp_c.wait()
                cp_wm.wait()
                c = c_v[...].astype(F32)
                wkv_v[48:64, :] = jnp.broadcast_to(c * jax.nn.sigmoid(c), (16, D)).astype(BF16)
                modulation(0, 2 * D)
                h_v[0] = (x1_v[...] * mod(1, 0, D, 4) + mod(0, 0, D, 4)).astype(BF16)
                for cp in (cp_wq, cp_wk, cp_wv):
                    cp.wait()
                _run(square_steps(w_v.at[0], wqt_v))
                pad = jnp.zeros((24 - Dh, D), F32)
                wkv_v[0:48, :] = _cat([wk_v[...].astype(F32), pad, wv_v[...].astype(F32), pad]).astype(BF16)

            pl.run_scoped(prologue, pltpu.VMEM((Dh, D), BF16), pltpu.VMEM((Dh, D), BF16),
                          pltpu.VMEM((1, D), BF16), pltpu.SemaphoreType.DMA((5,)))
            _loop(NQ, project)

            def first_tile(u):
                for cp in unit_copies(u):
                    cp.wait()

                @pl.when(u + 2 < NU)
                def _():
                    for cp in unit_copies(jnp.minimum(u + 2, NU - 1)):
                        cp.start()
                attend(u, NV0, None, weight_steps(u))
            _loop(NU, first_tile)

        pl.run_scoped(
            first_phase,
            pltpu.VMEM((2, D, D), BF16), pltpu.VMEM((3, 3, D, 4 * L), BF16),
            pltpu.VMEM((D, 6 * D), BF16), pltpu.VMEM((2, D, TQ), BF16), pltpu.VMEM((Dh, 8, L), F32),
            pltpu.VMEM((64, D), BF16), pltpu.VMEM((D // 4, 9 * L), U32), pltpu.VMEM((2, 2, 9, L // 2, L), U32),
            pltpu.SemaphoreType.DMA(()), pltpu.SemaphoreType.DMA((NQ,)), pltpu.SemaphoreType.DMA((3, 4)))

        bound = jnp.max(norm_v[0, 0:1, :], axis=1, keepdims=True) * norm_v[1, 0:1, :]
        ok = jnp.logical_and(bound <= SAFE_SCORE ** 2, norm_v[2, 0:1, :] <= SAFE_VALUE)
        safe = jnp.max(jnp.where(ok, 0.0, 1.0)) < 0.5

        def second_phase(p_v, hb_v, act_v, out_v, sems):
            def out_copy(t, half):
                rows = pl.ds(half * D // 2, D // 2)
                return pltpu.make_async_copy(out_v.at[t, rows], out_hbm.at[rows, _multiple(t, TQ)], sems.at[t, half])

            def early_scores(t, reuse, first_head, heads, first_key, keys, cycles):
                steps, operands = [], reuse(key_operand)
                for e in range(heads):
                    hh = first_head + e
                    queries = reuse(functools.partial(
                        query_operand, jnp.minimum((t + 1) * NG + (hh + 3) // 4, NQ * NG - 1), (e + 3) % 4))
                    for k0 in range(first_key, first_key + keys, 2 * KB):
                        def store(r, cols, s, k0=k0, hh=hh):
                            p_v[hh, k0 + r:k0 + r + 8, cols] = jnp.exp2(s)
                        steps += score_steps(operands, queries, (NB - NH + k0) // KB, store)
                return filler(cycles, steps)

            def project_heads(t):
                heads = o_v.at[pl.ds(t % 2 * H, H)]
                inv = [1.0 / heads[g:g + 8, Dh, :] for g in range(0, H, 8)]
                steps = []
                for pair in range(2):
                    cols = slice(2 * pair * L, 2 * (pair + 1) * L)
                    o = _cat([heads[hh, 0:Dh, cols] * inv[hh // 8][hh % 8:hh % 8 + 1, cols] for hh in range(H)])
                    for l, half, a in square_dot(wot_v, o.astype(BF16), (0, 1), filler(9 * D // 4, steps)):
                        r, c = half * D // 2, slice((2 * pair + l) * L, (2 * pair + l + 1) * L)
                        x1_v[r:r + D // 2, c] = x_v[t, r:r + D // 2, c].astype(F32) + mod(2, r, D // 2, 1) * a

                    def emit(r, norm, pair=pair):
                        h = [norm(r0) * mod(4, r0, 16, 2) + mod(3, r0, 16, 2) for r0 in (r, r + D // 2)]
                        y = _words(_cat(_strassen_rhs([[hk[:, 0:L], hk[:, L:]] for hk in h]), 1))
                        for i in range(7):
                            hb_v[i, r // 2:r // 2 + 8, pair * L:(pair + 1) * L] = y[:, i * L:(i + 1) * L]
                    steps = _norm_steps(lambda r, n, cols=cols: x1_v[r:r + n, cols], D, emit, range(0, D // 2, 16))
                _run(steps)

            def gate_up(t, it):
                room = ((96, 80, 96, 96, 80, 80, 80), (96, 60, 96, 96, 60, 60, 60))
                fill = early_scores(t, functools.cache, it * (H // GI), H // GI, 0, NH_UP,
                                    UG * (7 * 24 + 2 * sum(room[0] + room[1])))
                for block in range(UG):
                    rows = _multiple(it * UG + block, RB // 2)
                    shared = [[None] * 2 for _ in range(2)]
                    for i in range(7):
                        m = _dot(_bf16(ws_v[i, rows, :]), _bf16(hb_v[i, 80:144, :]))
                        fill.tick(m, 24)
                        _strassen_add(shared, i, m)
                    acts = []
                    for n in range(4):
                        c = [list(r) for r in shared]
                        for at, i in enumerate((2, 4, 0, 1, 5, 3, 6)):
                            rhs = [hb_v[i, 0:64, :]] + [
                                hb_v[i, pl.ds(64 if m == n else 80 + 16 * m, 16), :] for m in range(4)]
                            m = _dot(_bf16(wa_v[i, n, rows, :]), _bf16(_cat(rhs)))
                            fill.tick(m, room[n % 2][at])
                            _strassen_add(c, i, m)
                        acts.append([_cat([_swiglu(c[row][k][r:r + 16], c[row][k][r + 16:r + 32])
                                          for r in range(0, RB, 32) for row in range(2)]) for k in range(2)])
                        if n % 2 == 1:
                            for i, y in enumerate(_strassen_rhs(acts[n - 1:])):
                                act_v[i, n // 2, _multiple(it * UG + block, RB), :] = y

            def down(t):
                fill = early_scores(t, lambda f: f, 0, H, NH_UP, NH_DOWN, 49 * NU * D // 16)
                y = [[[[None] * 2 for _ in range(2)] for _ in range(2)] for _ in range(2)]
                for i in (2, 3, 4, 1, 0, 6, 5):
                    c = [[None] * 2 for _ in range(2)]
                    for k in range(7):
                        acc = None
                        for u0, u1 in ((0, 4), (4, 5), (5, NU)):
                            b = _strassen_rhs([[act_v[i, r, u0 * L:u1 * L, n * L:(n + 1) * L] for n in range(2)]
                                               for r in range(2)])[k]
                            m = _dot(_bf16(_cat([wd_v[7 * i + k, u] for u in range(u0, u1)], 1)), b.astype(BF16))
                            fill.tick(m, (u1 - u0) * D // 16)
                            acc = m if acc is None else acc + m
                        _strassen_add(c, k, acc)
                    for r in range(2):
                        for n in range(2):
                            _strassen_add(y[r][n], i, c[r][n])
                    if i in (6, 5):
                        half = 6 - i
                        rows = slice(half * D // 2, (half + 1) * D // 2)
                        ffn = _cat([_cat([y[r][n // 2][half][n % 2] for n in range(4)], 1) for r in range(2)])
                        out_v[t, rows, :] = (x1_v[rows, :] + mod(5, rows.start, D // 2, 4) * ffn).astype(BF16)
                        out_copy(t, half).start()

            def tile(t):
                @pl.when(safe)
                def _():
                    _loop(jnp.where(t == 0, 0, jnp.where(t == NQ - 1, NG - 1, NG)),
                          lambda g: attend(t * NG + 1 + g, NV1, lambda j: p_v.at[4 * g + j]))

                    def last_head(_):
                        o_v[2 * H - 1] = sum(weigh_values(1, c, p_v.at[H - 4], True) for c in range(NC))
                    _loop(jnp.where(t == NQ - 1, 1, 0), last_head)

                @pl.when(jnp.logical_not(safe))
                def _():
                    _loop(4 * H, lambda n: attend_with_max(t, n))

                project_heads(t)
                _loop(GI, lambda it: gate_up(t, it))
                down(t)

            _loop(NQ, tile)
            for t in range(NQ):
                for half in range(2):
                    out_copy(t, half).wait()

        pl.run_scoped(
            second_phase,
            pltpu.VMEM((H, NH, TQ), F32), pltpu.VMEM((7, D // 4, 2 * L), U32),
            pltpu.VMEM((7, 2, NU * L, 2 * L), F32), pltpu.VMEM((NQ, D, TQ), BF16),
            pltpu.SemaphoreType.DMA((NQ, 2)))

    scratch = [
        pltpu.VMEM((NQ, D, TQ), BF16),
        pltpu.VMEM((D, TQ), F32),
        pltpu.VMEM((6 * D, L), F32),
        pltpu.VMEM((3, 8, TQ), F32),
        pltpu.VMEM((16, L), jnp.int32),
        pltpu.VMEM((D // 4, 9 * L), U32),
        pltpu.VMEM((NQ * NG, 4 * Dh, 3 * TQ), F32),
        pltpu.VMEM((S // 2, 32), U32),
        pltpu.VMEM((NB // KB // 2, 64, 16, L), F32),
        pltpu.VMEM((NC, 24, L), F32),
        pltpu.VMEM((2, S, TQ), F32),
        pltpu.VMEM((2 * H, 24, TQ), F32),
        pltpu.VMEM((7, 4, NU * L // 2, 2 * L), U32),
        pltpu.VMEM((7, NU * L // 2, L), U32),
        pltpu.VMEM((51, NU, D // 8, L), U32),
    ]
    return kernel, scratch


@jax.jit
def pallas_adaLN_cond__grouped_kv_mqa__swiglu_ffn__prompt_kernel(
    A_x: jax.Array,
    A_wq: jax.Array,
    A_wk: jax.Array,
    A_wv: jax.Array,
    A_wo: jax.Array,
    B_x: jax.Array,
    B_w_gate: jax.Array,
    B_w_up: jax.Array,
    B_w_down: jax.Array,
    c: jax.Array,
    w_mod: jax.Array,
):
    del B_x
    _, S, D = A_x.shape
    kernel, scratch = _make_kernel(S, D, B_w_gate.shape[1])
    out_t = pl.pallas_call(
        kernel,
        in_specs=[pl.BlockSpec(memory_space=pl.ANY)] * 10,
        out_specs=pl.BlockSpec(memory_space=pl.ANY),
        out_shape=jax.ShapeDtypeStruct((D, S), A_x.dtype),
        scratch_shapes=scratch,
        compiler_params=pltpu.CompilerParams(vmem_limit_bytes=122 * 2 ** 20),
        name="adaln_block",
    )(A_x.reshape(S, D).T, A_wq, A_wk.T, A_wv.T, A_wo, B_w_gate, B_w_up, B_w_down.T, c, w_mod)
    return out_t.T.reshape(1, S, D)
```
